```python
import jax
import jax.numpy as jnp

def _softmax(x, axis=-1):
    return jax.nn.softmax(x, axis=axis)
def _gelu(x):
    return jax.nn.gelu(x, approximate=True)
def _silu(x):
    return jax.nn.silu(x)
def _sigmoid(x):
    return jax.nn.sigmoid(x)
def _layernorm(x, axis=-1, eps=1e-5):
    m = jnp.mean(x, axis=axis, keepdims=True)
    v = jnp.var(x, axis=axis, keepdims=True)
    return (x - m) / jnp.sqrt(v + eps)
def _scatter_add(tgt, idx, src, axis=0):
    return tgt.at[idx].add(src)
def _segment_sum(src, seg, n):
    return jax.ops.segment_sum(src, seg, n)
class _Rng:
    def __init__(self, key):
        self._k = key
    def _next(self):
        self._k, sub = jax.random.split(self._k)
        return sub
    def normal(self, shape):
        return jax.random.normal(self._next(), shape, dtype=jnp.bfloat16)
    def randint(self, lo, hi, shape):
        return jax.random.randint(self._next(), shape, lo, hi, dtype=jnp.int32)
    def uniform(self, shape, lo=0.0, hi=1.0):
        return jax.random.uniform(self._next(), shape, jnp.bfloat16, lo, hi)
    def permutation(self, n):
        return jax.random.permutation(self._next(), n)


kernel_name = 'standalone__structured_sparse_n_m__ragged'

def setup_inputs():
    _rng = _Rng(jax.random.key(int.from_bytes(__import__("os").urandom(4), "little")))
    _w = (lambda a: (lambda t: t.astype(jnp.bfloat16) if jnp.issubdtype(t.dtype, jnp.floating) else t)(jnp.asarray(a)))
    B, S, D = 16, 4096, 576
    assert D % 4 == 0, "d_model must be divisible by M=4 for 2:4 sparsity"
    return {
        "x": _w((lambda *s: _rng.normal(s) * 0.05)(B, S, D)),
        "w": _w((lambda *s: _rng.normal(s) * 0.05)(D, D)),
        "b": _w((lambda *s: _rng.normal(s) * 0.05)(D)),
    }

def reference(x, w, b):
    B, S, D = x.shape
    N, M = 2, 4
    G = D // M
    wg = w.reshape(G, M, D)
    mag = jnp.abs(wg)
    order = jnp.argsort(mag, 1)
    thr = jnp.take_along_axis(mag, order[:, M - N:M - N + 1, :], 1)
    mask = (lambda x, dt: x.astype(dt))(mag >= thr, w.dtype)
    wp = (wg * mask).reshape(D, D)
    return jnp.einsum("bsd,df->bsf", x, wp) + b
```

```python
import jax
import jax.numpy as jnp
from jax import lax
import jax.experimental.pallas as pl
import jax.experimental.pallas.tpu as pltpu

KB = 64
CH = 256
RHO = 2.0
SLOPES = ((1.0, 1.0), (RHO, 1.0), (1.0, RHO), (1 / RHO, RHO))
PASSES = ("1Q", "rQ", "iQ", "phi", "1P", "rP", "iP", "psi",
          "p1", "pr", "n11a", "n11b", "q1", "qr", "n22a", "n22b")

IN_FIRST = (1, 1, 2, 4, 8)
WRITE_FROM = 124
RING = 9


def _prune_packed(u):
    mate = lax.broadcasted_iota(jnp.int32, u.shape, 0) ^ 1
    lo = pltpu.bitcast((u << 16) & 0x7FFFFFFF, jnp.float32)
    hi = pltpu.bitcast(u & 0x7FFF0000, jnp.float32)
    big, small = jnp.maximum(lo, hi), jnp.minimum(lo, hi)
    nbig = jnp.take_along_axis(big, mate, axis=0, mode="promise_in_bounds")
    nsmall = jnp.take_along_axis(small, mate, axis=0, mode="promise_in_bounds")
    thr = jnp.maximum(jnp.minimum(big, nbig), jnp.maximum(small, nsmall))
    return u & (jnp.where(lo < thr, 0, 0xFFFF) | jnp.where(hi < thr, 0, -65536))


def _prune(w):
    u = pltpu.bitcast(w, jnp.int32)
    parts = [_prune_packed(u[8 * i:8 * i + 8]) for i in range(u.shape[0] // 8)]
    return pltpu.bitcast(jnp.concatenate(parts, axis=0), jnp.bfloat16)


def _weight_tiles(wp):
    wt = wp.T.astype(jnp.float32)
    half = wt.shape[0] // 2
    a = lambda i, k: wt[i * half:(i + 1) * half, KB * k:KB * (k + 1)]
    terms = []
    for n, (s, _) in enumerate(SLOPES):
        a11, a12, a21, a22 = a(0, n), a(0, 4 + n), a(1, n) * (1 / s), a(1, 4 + n) * (1 / s)
        terms.append([a11 + a22, a21 + a22, a11, a22, a11 + a12, a21 - a11, a12 - a22])
    A, B, C, D = terms
    u = (a(1, 8) - a(0, 8) * (1 / RHO)) * (1 / (RHO - 1 / RHO))
    v = (a(0, 8) * RHO - a(1, 8)) * (1 / (RHO - 1 / RHO))
    pairs = {
        "phi": (A[0], D[0]), "psi": (B[0], C[0]),
        "q1": (A[1], B[1] * RHO), "qr": (C[1], D[1] * (1 / RHO)),
        "1P": (A[2], C[2] * RHO), "rP": (B[2], u), "iP": (D[2] * RHO, v),
        "1Q": (A[3], C[3]), "rQ": (B[3], u), "iQ": (D[3], v),
        "p1": (A[4], B[4]), "pr": (C[4], D[4]),
        "n22a": (A[5], B[5] * RHO), "n22b": (C[5] * RHO, D[5]),
        "n11a": (A[6], B[6]), "n11b": (C[6], D[6]),
    }
    return {p: jnp.concatenate(pairs[p], axis=1).astype(jnp.bfloat16) for p in PASSES}


def _token_tiles(x):
    b = lambda k, j: x[KB * k:KB * (k + 1), 128 * j:128 * (j + 1)]
    terms = []
    for n, (_, t) in enumerate(SLOPES):
        b11, b12, b21, b22 = b(n, 0), b(n, 1), b(4 + n, 0), b(4 + n, 1)
        if t != 1.0:
            b12, b22 = b12 * (1 / t), b22 * (1 / t)
        terms.append([b11 + b22, b11, b12 - b22, b21 - b11, b22, b11 + b12, b21 + b22])
    A, B, C, D = terms
    pairs = {
        "phi": (A[0], D[0]), "psi": (B[0], C[0]),
        "q1": (A[1], B[1]), "qr": (C[1], D[1]),
        "1P": (A[2], C[2]), "rP": (B[2], b(8, 1)), "iP": (D[2], b(8, 1)),
        "1Q": (A[3], C[3]), "rQ": (B[3], b(8, 0)), "iQ": (D[3], b(8, 0)),
        "p1": (A[4], B[4]), "pr": (C[4], D[4]),
        "n22a": (A[5], B[5]), "n22b": (C[5], D[5]),
        "n11a": (A[6], B[6]), "n11b": (C[6], D[6]),
    }
    return {p: jnp.concatenate(pairs[p], axis=0).astype(jnp.bfloat16) for p in PASSES}


def _kernel(x_hbm, w_hbm, b_hbm, o_hbm, xbuf, obuf, wbuf, bbuf, lhs, bias, isem, osem):
    NB, _, S = x_hbm.shape
    F = w_hbm.shape[1]
    H = F // 2
    CPB = S // CH
    first = [(sum(IN_FIRST[:j]), n) for j, n in enumerate(IN_FIRST)]
    nf = len(first)

    def icopy_first(j):
        cols = pl.ds(first[j][0] * CH, first[j][1] * CH)
        return pltpu.make_async_copy(x_hbm.at[0, :, cols], xbuf.at[0, :, cols], isem.at[j])

    def icopy(bi):
        return pltpu.make_async_copy(x_hbm.at[bi], xbuf.at[bi], isem.at[nf + bi - 1])

    def ring(bi):
        return jnp.where(bi >= RING, bi - RING, bi)

    def ostart(bi, g):
        pltpu.make_async_copy(
            obuf.at[ring(bi), g], o_hbm.at[bi, :, pl.ds(g * CH, CH)], osem.at[ring(bi)]).start()

    def owait(slot):
        pltpu.make_async_copy(obuf.at[slot], obuf.at[slot], osem.at[slot]).wait()

    wcp = pltpu.make_async_copy(w_hbm, wbuf, isem.at[nf + NB - 1])
    bcp = pltpu.make_async_copy(b_hbm, bbuf, isem.at[nf + NB])
    wcp.start()
    bcp.start()
    for j in range(nf):
        icopy_first(j).start()
    for bi in range(1, NB):
        icopy(bi).start()
    wcp.wait()
    bcp.wait()
    tiles = _weight_tiles(_prune(wbuf[...]))
    for i, p in enumerate(PASSES):
        lhs[i] = pltpu.bitcast(tiles[p], jnp.int32)
    bias[...] = jnp.broadcast_to(bbuf[...].reshape(1, F).astype(jnp.float32), (128, F)).T

    def compute(bi, g):
        slot = ring(bi)
        rhs = _token_tiles(xbuf[bi, :, pl.ds(g * CH, CH)].astype(jnp.float32))

        def mm(p):
            return jnp.dot(pltpu.bitcast(lhs[PASSES.index(p)], jnp.bfloat16), rhs[p],
                           preferred_element_type=jnp.float32)

        def store(rows, left, right):
            obuf[slot, g, rows, :] = jnp.concatenate([left, right], axis=1).astype(obuf.dtype)

        m1q, mrq, miq, phi = mm("1Q"), mm("rQ"), mm("iQ"), mm("phi")
        c11 = (m1q + mrq) + (miq + phi)
        c21 = m1q + mrq * RHO + miq * (1 / RHO)
        m1p, mrp, mip, psi = mm("1P"), mm("rP"), mm("iP"), mm("psi")
        c12 = m1p + mrp + mip
        c22 = (m1p + phi) + (mrp + psi) * RHO + mip * (1 / RHO)
        mp1, mpr, n11a, n11b = mm("p1"), mm("pr"), mm("n11a"), mm("n11b")
        b1, b2 = bias[0:H], bias[H:F]
        c12 = (c12 + b1) + mp1 + mpr * RHO
        c11 = ((c11 + psi) + b1) + (n11a + n11b) - (mp1 + mpr)
        store(pl.ds(0, H), c11, c12)
        mq1, mqr, n22a, n22b = mm("q1"), mm("qr"), mm("n22a"), mm("n22b")
        c21 = (c21 + b2) + (mq1 + mqr)
        c22 = (c22 + b2) + (n22a + n22b) - (mq1 + mqr * RHO)
        store(pl.ds(H, H), c21, c22)

    def body(bi, carry):
        for g in range(CPB):
            for j in range(nf):
                if first[j][0] == g:
                    pl.when(bi == 0)(lambda: icopy_first(j).wait())
            if g == 0:
                pl.when(bi > 0)(lambda: icopy(bi).wait())
                pl.when(bi >= RING)(lambda: owait(bi - RING))
            compute(bi, g)
            step = bi * CPB + g
            for e in range(2):
                q = 2 * (g - WRITE_FROM) + e
                chunk = 2 * CPB * bi + q
                pl.when((chunk >= 0) & (chunk <= step))(
                    lambda: ostart(2 * bi + q // CPB, q % CPB))
            if (NB - 1) * CPB + g > 2 * WRITE_FROM:
                pl.when(step > 2 * WRITE_FROM)(lambda: ostart(bi, g))
        return carry

    assert 2 * WRITE_FROM <= NB * CPB
    lax.fori_loop(0, NB, body, 0)
    for bi in range(NB - RING, NB):
        owait(bi % RING)


@jax.jit
def pallas_standalone__structured_sparse_n_m__ragged_kernel(
    x: jax.Array,
    w: jax.Array,
    b: jax.Array,
):
    B, S, D = x.shape
    F = w.shape[1]
    out = pl.pallas_call(
        _kernel,
        in_specs=[pl.BlockSpec(memory_space=pl.ANY)] * 3,
        out_specs=pl.BlockSpec(memory_space=pl.ANY),
        out_shape=jax.ShapeDtypeStruct((B, F, S), x.dtype),
        scratch_shapes=[
            pltpu.VMEM((B, D, S), x.dtype),
            pltpu.VMEM((RING, S // CH, F, CH), x.dtype),
            pltpu.VMEM((D, F), w.dtype),
            pltpu.VMEM((F,), b.dtype),
            pltpu.VMEM((len(PASSES), F // 4, 128), jnp.int32),
            pltpu.VMEM((F, 128), jnp.float32),
            pltpu.SemaphoreType.DMA((len(IN_FIRST) + B + 1,)),
            pltpu.SemaphoreType.DMA((RING,)),
        ],
        compiler_params=pltpu.CompilerParams(
            vmem_limit_bytes=126 * 1024 * 1024,
            disable_bounds_checks=True,
            flags={"XLA_TPU_RESCHEDULE_DMA_DONES": True},
        ),
    )(jnp.transpose(x, (0, 2, 1)), w, b)
    return jnp.transpose(out, (0, 2, 1))
```

```python
import jax
import jax.numpy as jnp
from jax import lax
import jax.experimental.pallas as pl
import jax.experimental.pallas.tpu as pltpu

KB = 64
CH = 256
GS = 4
RHO = 2.0
SLOPES = ((1.0, 1.0), (RHO, 1.0), (1.0, RHO), (1 / RHO, RHO))
PASSES = ("1Q", "rQ", "iQ", "phi", "1P", "rP", "iP", "psi", "p1", "pr", "q1", "qr")
DIAG = ("n11", "n22")

PACED = 128
WRITE_FROM = 123
WRITE_RATE = 8
WRITE_TAIL = {14: (8, 8), 15: (4, 4, 4, 2, 2)}
RING = 9


def _prune_packed(u):
    mate = lax.broadcasted_iota(jnp.int32, u.shape, 0) ^ 1
    lo = pltpu.bitcast((u << 16) & 0x7FFFFFFF, jnp.float32)
    hi = pltpu.bitcast(u & 0x7FFF0000, jnp.float32)
    big, small = jnp.maximum(lo, hi), jnp.minimum(lo, hi)
    nbig = jnp.take_along_axis(big, mate, axis=0, mode="promise_in_bounds")
    nsmall = jnp.take_along_axis(small, mate, axis=0, mode="promise_in_bounds")
    thr = jnp.maximum(jnp.minimum(big, nbig), jnp.maximum(small, nsmall))
    return u & (jnp.where(lo < thr, 0, 0xFFFF) | jnp.where(hi < thr, 0, -65536))


def _prune(w):
    u = pltpu.bitcast(w, jnp.int32)
    parts = [_prune_packed(u[8 * i:8 * i + 8]) for i in range(u.shape[0] // 8)]
    return pltpu.bitcast(jnp.concatenate(parts, axis=0), jnp.bfloat16)


def _strassen_left(a11, a12, a21, a22):
    return [a11 + a22, a21 + a22, a11, a22, a11 + a12, a21 - a11, a12 - a22]


def _strassen_right(b11, b12, b21, b22):
    return [b11 + b22, b11, b12 - b22, b21 - b11, b22, b11 + b12, b21 + b22]


def _weight_terms(wp):
    wt = wp.T.astype(jnp.float32)
    half = wt.shape[0] // 2
    a = lambda i, k: wt[i * half:(i + 1) * half, KB * k:KB * (k + 1)]
    A, B, C, D = [_strassen_left(a(0, n), a(0, 4 + n), a(1, n) * (1 / s), a(1, 4 + n) * (1 / s))
                  for n, (s, _) in enumerate(SLOPES)]
    u = (a(1, 8) - a(0, 8) * (1 / RHO)) * (1 / (RHO - 1 / RHO))
    v = (a(0, 8) * RHO - a(1, 8)) * (1 / (RHO - 1 / RHO))
    pairs = {
        "phi": (A[0], D[0]), "psi": (B[0], C[0]),
        "q1": (A[1], B[1] * RHO), "qr": (C[1], D[1] * (1 / RHO)),
        "1P": (A[2], C[2] * RHO), "rP": (B[2], u), "iP": (D[2] * RHO, v),
        "1Q": (A[3], C[3]), "rQ": (B[3], u), "iQ": (D[3], v),
        "p1": (A[4], B[4]), "pr": (C[4], D[4]),
        "n22a": (A[5], B[5] * RHO), "n22b": (C[5] * RHO, D[5]),
        "n11a": (A[6], B[6]), "n11b": (C[6], D[6]),
    }
    return {p: jnp.concatenate(v, axis=1) for p, v in pairs.items()}


def _token_terms(x):
    b = lambda k, j: x[KB * k:KB * (k + 1), 128 * j:128 * (j + 1)]
    terms = []
    for n, (_, t) in enumerate(SLOPES):
        b11, b12, b21, b22 = b(n, 0), b(n, 1), b(4 + n, 0), b(4 + n, 1)
        if t != 1.0:
            b12, b22 = b12 * (1 / t), b22 * (1 / t)
        terms.append(_strassen_right(b11, b12, b21, b22))
    A, B, C, D = terms
    pairs = {
        "phi": (A[0], D[0]), "psi": (B[0], C[0]),
        "q1": (A[1], B[1]), "qr": (C[1], D[1]),
        "1P": (A[2], C[2]), "rP": (B[2], b(8, 1)), "iP": (D[2], b(8, 1)),
        "1Q": (A[3], C[3]), "rQ": (B[3], b(8, 0)), "iQ": (D[3], b(8, 0)),
        "p1": (A[4], B[4]), "pr": (C[4], D[4]),
        "n22a": (A[5], B[5]), "n22b": (C[5], D[5]),
        "n11a": (A[6], B[6]), "n11b": (C[6], D[6]),
    }
    return {p: jnp.concatenate(v, axis=0) for p, v in pairs.items()}


def _write_plan(nb, spb):
    copies = []
    for b in range(nb):
        first = 0
        for n in WRITE_TAIL.get(b, (spb,)):
            ready = b * spb + first + n - 1
            copies += [(ready, b, p, c) for p in range(8) for c in range(first, first + n, 2)]
            first += n
    issued = {}
    step, used = WRITE_FROM, -WRITE_RATE
    for ready, b, p, c in copies:
        if used == WRITE_RATE:
            step, used = step + 1, 0
        if ready > step:
            step, used = ready, WRITE_RATE * (step - ready)
        used += 1
        it, g = divmod(min(step, nb * spb - 1), spb)
        issued.setdefault((g, b - 2 * it, p, c), []).append(it)
    plan = {}
    for (g, db, p, c), its in issued.items():
        for lo in [it for it in its if it - 1 not in its]:
            hi = min(it for it in its if it >= lo and it + 1 not in its)
            plan.setdefault(g, {}).setdefault((lo, hi), []).append((db, p, c))
    return plan


def _kernel(x_hbm, w_hbm, b_hbm, o_hbm, xbuf, obuf, wbuf, bbuf, lhs, lhs_diag, bias, isem, osem):
    NB, D, S = x_hbm.shape
    F = w_hbm.shape[1]
    H = F // 2
    SPB = S // CH
    everything = slice(None)

    def xcopy(bi, rows, cols, sem):
        return pltpu.make_async_copy(x_hbm.at[bi, rows, cols], xbuf.at[bi, rows, cols], isem.at[sem])

    def background():
        return xcopy(pl.ds(PACED // SPB, NB - PACED // SPB), everything, everything, 2)

    def ring(bi):
        return jnp.where(bi >= RING, bi - RING, bi)

    def ostart(bi, phase, step):
        cols = pl.ds(step * CH, 2 * CH)
        pltpu.make_async_copy(obuf.at[ring(bi), :, phase, :, cols], o_hbm.at[bi, :, phase, :, cols],
                              osem.at[ring(bi)]).start()

    def owait(slot):
        pltpu.make_async_copy(obuf.at[slot], obuf.at[slot], osem.at[slot]).wait()

    wcp = pltpu.make_async_copy(w_hbm, wbuf, isem.at[3])
    bcp = pltpu.make_async_copy(b_hbm, bbuf, isem.at[4])
    wcp.start()
    bcp.start()
    for j in range(2):
        xcopy(0, everything, pl.ds(j * GS * CH, GS * CH), j).start()
    background().start(priority=1)
    wcp.wait()
    bcp.wait()
    wt = _weight_terms(_prune(wbuf[...]))
    for i, p in enumerate(PASSES):
        lhs[i] = pltpu.bitcast(wt[p].astype(jnp.bfloat16), jnp.int32)
    for k, n in enumerate(DIAG):
        la, lb = wt[n + "a"], wt[n + "b"]
        for i, m in enumerate(_strassen_left(la[:H // 2], lb[:H // 2], la[H // 2:], lb[H // 2:])):
            lhs_diag[7 * k + i] = pltpu.bitcast(m.astype(jnp.bfloat16), jnp.int32)
    bias[...] = jnp.broadcast_to(bbuf[...].reshape(1, F).astype(jnp.float32), (128, F)).T

    def dot(left_words, right):
        return jnp.dot(pltpu.bitcast(left_words, jnp.bfloat16), right.astype(jnp.bfloat16),
                       preferred_element_type=jnp.float32)

    def terms(bi, step):
        return _token_terms(xbuf[bi, :, pl.ds(step * CH, CH)].astype(jnp.float32))

    plan = _write_plan(NB, SPB)

    def group(bi, g):
        sem = g // GS % 2
        pl.when(bi * SPB + g < PACED)(lambda: xcopy(0, everything, pl.ds(0, GS * CH), sem).wait())
        if g == 0:
            pl.when(bi == PACED // SPB)(lambda: background().wait())
            pl.when(bi >= RING)(lambda: owait(bi - RING))
        pieces = list(range(4 * GS))

        def fetch():
            i = pieces.pop(0)
            step = g + 2 * GS + i // 4
            pl.when(bi * SPB + g + 2 * GS < PACED)(
                lambda: xcopy(bi + step // SPB, pl.ds(i % 4 * (D // 4), D // 4),
                              pl.ds(step % SPB * CH, CH), sem).start())

        diag = {}
        for e in range(0, GS, 2):
            for k, n in enumerate(DIAG):
                fetch()
                t0, t1 = terms(bi, g + e), terms(bi, g + e + 1)
                r = _strassen_right(t0[n + "a"], t1[n + "a"], t0[n + "b"], t1[n + "b"])
                m = {i: dot(lhs_diag[7 * k + i], r[i]) for i in (0, 3, 4, 6, 2, 1, 5)}
                diag[n, e] = jnp.concatenate([(m[0] + m[3]) + (m[6] - m[4]), m[1] + m[3]], axis=0)
                diag[n, e + 1] = jnp.concatenate([m[2] + m[4], (m[0] - m[1]) + (m[2] + m[5])], axis=0)

        for e in range(GS):
            def passes(*names):
                fetch()
                t = terms(bi, g + e)
                return [dot(lhs[PASSES.index(p)], t[p]) for p in names]

            m1q, mrq, miq, phi = passes("1Q", "rQ", "iQ", "phi")
            c11 = (m1q + mrq) + (miq + phi) + diag["n11", e]
            c21 = m1q + mrq * RHO + miq * (1 / RHO)
            c22 = diag["n22", e] + phi
            m1p, mrp, mip, psi = passes("1P", "rP", "iP", "psi")
            c12 = m1p + mrp + mip
            c22 = (c22 + m1p) + (mrp + psi) * RHO + mip * (1 / RHO)
            mp1, mpr, mq1, mqr = passes("p1", "pr", "q1", "qr")
            b1, b2 = bias[0:H], bias[H:F]
            c12 = (c12 + b1) + mp1 + mpr * RHO
            c11 = ((c11 + psi) + b1) - (mp1 + mpr)
            c21 = (c21 + b2) + (mq1 + mqr)
            c22 = (c22 + b2) - (mq1 + mqr * RHO)

            slot, cols = ring(bi), pl.ds((g + e) * CH, CH)
            top = jnp.concatenate([c11, c12], axis=1)
            obuf[slot, 0:4, :, :, cols] = top[:256].reshape(4, 8, 8, CH).astype(obuf.dtype)
            obuf[slot, 4, 0:4, :, cols] = top[256:].reshape(4, 8, CH).astype(obuf.dtype)
            bottom = jnp.concatenate([c21, c22], axis=1)
            obuf[slot, 4, 4:8, :, cols] = bottom[:32].reshape(4, 8, CH).astype(obuf.dtype)
            obuf[slot, 5:9, :, :, cols] = bottom[32:].reshape(4, 8, 8, CH).astype(obuf.dtype)

            for (lo, hi), copies in plan.get(g + e, {}).items():
                for i in range(0, len(copies), 4):
                    @pl.when((bi >= lo) & (bi <= hi))
                    def _():
                        for db, phase, step in copies[i:i + 4]:
                            ostart(2 * bi + db, phase, step)

    def body(bi, carry):
        for g in range(0, SPB, GS):
            group(bi, g)
        return carry

    lax.fori_loop(0, NB, body, 0)
    for bi in range(NB - RING, NB):
        owait(bi % RING)


@jax.jit
def pallas_standalone__structured_sparse_n_m__ragged_kernel(
    x: jax.Array,
    w: jax.Array,
    b: jax.Array,
):
    B, S, D = x.shape
    F = w.shape[1]
    out = pl.pallas_call(
        _kernel,
        in_specs=[pl.BlockSpec(memory_space=pl.ANY)] * 3,
        out_specs=pl.BlockSpec(memory_space=pl.ANY),
        out_shape=jax.ShapeDtypeStruct((B, F // 64, 8, 8, S), x.dtype),
        scratch_shapes=[
            pltpu.VMEM((B, D, S), x.dtype),
            pltpu.VMEM((RING, F // 64, 8, 8, S), x.dtype),
            pltpu.VMEM((D, F), w.dtype),
            pltpu.VMEM((F,), b.dtype),
            pltpu.VMEM((len(PASSES), F // 4, 128), jnp.int32),
            pltpu.VMEM((7 * len(DIAG), F // 8, 128), jnp.int32),
            pltpu.VMEM((F, 128), jnp.float32),
            pltpu.SemaphoreType.DMA((5,)),
            pltpu.SemaphoreType.DMA((RING,)),
        ],
        compiler_params=pltpu.CompilerParams(
            vmem_limit_bytes=126 * 1024 * 1024,
            disable_bounds_checks=True,
            disable_semaphore_checks=True,
            flags={"XLA_TPU_RESCHEDULE_DMA_DONES": True},
        ),
    )(jnp.transpose(x, (0, 2, 1)), w, b)
    return jnp.transpose(out.reshape(B, F, S), (0, 2, 1))
```

```python
import jax
import jax.numpy as jnp
from jax import lax
import jax.experimental.pallas as pl
import jax.experimental.pallas.tpu as pltpu

KB = 64
CH = 256
GROUP = 4
UNIT = 8
UNROLL = 2

RHO = 2.0
T_SCALE = (1.0, 1.0, RHO, RHO)
PASSES = ("1Q", "rQ", "iQ", "phi", "1P", "rP", "iP", "psi", "p1", "pr", "q1", "qr")
DIAG = ("n11", "n22")
PRODUCTS = {
    "phi": ((0, 0), (3, 0)), "psi": ((2, 0), (1, 0)),
    "q1": ((0, 1), (1, 1)), "qr": ((2, 1), (3, 1)),
    "1P": ((0, 2), (2, 2)), "rP": ((8, 1), (1, 2)), "iP": ((8, 1), (3, 2)),
    "1Q": ((0, 3), (2, 3)), "rQ": ((8, 0), (1, 3)), "iQ": ((8, 0), (3, 3)),
    "p1": ((0, 4), (1, 4)), "pr": ((2, 4), (3, 4)),
    "n22a": ((0, 5), (1, 5)), "n22b": ((2, 5), (3, 5)),
    "n11a": ((0, 6), (1, 6)), "n11b": ((2, 6), (3, 6)),
}

PACED = 128
PACED_EXTRA = 5
WRITE_FROM = 122
WRITE_TAIL = {14: (8, 8), 15: (4, 4, 4, 1, 1, 1, 1)}
RING = 9


def _prune_packed(u):
    mate = lax.broadcasted_iota(jnp.int32, u.shape, 0) ^ 1
    lo = pltpu.bitcast((u << 16) & 0x7FFFFFFF, jnp.float32)
    hi = pltpu.bitcast(u & 0x7FFF0000, jnp.float32)
    big, small = jnp.maximum(lo, hi), jnp.minimum(lo, hi)
    nbig = jnp.take_along_axis(big, mate, axis=0, mode="promise_in_bounds")
    nsmall = jnp.take_along_axis(small, mate, axis=0, mode="promise_in_bounds")
    thr = jnp.maximum(jnp.minimum(big, nbig), jnp.maximum(small, nsmall))
    return u & (jnp.where(lo < thr, 0, 0xFFFF) | jnp.where(hi < thr, 0, -65536))


def _prune(w):
    u = pltpu.bitcast(w, jnp.int32)
    parts = [_prune_packed(u[8 * i:8 * i + 8]) for i in range(u.shape[0] // 8)]
    return pltpu.bitcast(jnp.concatenate(parts, axis=0), jnp.bfloat16)


def _strassen_left(a11, a12, a21, a22):
    return [a11 + a22, a21 + a22, a11, a22, a11 + a12, a21 - a11, a12 - a22]


def _strassen_right(b11, b12, b21, b22):
    return [b11 + b22, b11, b12 - b22, b21 - b11, b22, b11 + b12, b21 + b22]


def _left_operands(wt):
    h = wt[0].shape[0] // 2
    low = lax.broadcasted_iota(jnp.int32, (h, 128), 1) < KB
    mix = lambda a, b: jnp.where(low, a, b)
    per_block = lambda a, b: jnp.where(low[0:1], a, b)
    inv_ab, inv_cd = per_block(1.0, 1 / RHO), per_block(1.0, RHO)
    ab = _strassen_left(wt[0][:h], wt[2][:h], wt[0][h:] * inv_ab, wt[2][h:] * inv_ab)
    cd = _strassen_left(wt[1][:h], wt[3][:h], wt[1][h:] * inv_cd, wt[3][h:] * inv_cd)
    u = (wt[4][h:] - wt[4][:h] * (1 / RHO)) * (1 / (RHO - 1 / RHO))
    v = (wt[4][:h] * RHO - wt[4][h:]) * (1 / (RHO - 1 / RHO))
    cd2 = cd[2] * RHO
    return {
        "phi": mix(ab[0], cd[0]), "psi": mix(cd[0], ab[0]),
        "q1": ab[1] * per_block(1.0, RHO), "qr": cd[1] * per_block(1.0, 1 / RHO),
        "1P": mix(ab[2], pltpu.roll(cd2, KB, 1)), "rP": mix(u, ab[2]), "iP": mix(v, cd2),
        "1Q": mix(ab[3], pltpu.roll(cd[3], KB, 1)), "rQ": mix(u, ab[3]), "iQ": mix(v, cd[3]),
        "p1": ab[4], "pr": cd[4],
        "n22a": ab[5] * per_block(1.0, RHO), "n22b": cd[5] * per_block(RHO, 1.0),
        "n11a": ab[6], "n11b": cd[6],
    }


def _write_plan(nb, spb):
    plan, step, sent = {}, WRITE_FROM, 0
    for b in range(nb):
        first = 0
        for n in WRITE_TAIL.get(b, (spb,)):
            ready = b * spb + first + n - 1
            if n == 1:
                copies = [(b, None, first, 1)]
            else:
                copies = [(b, p, c, 2) for p in range(8) for c in range(first, first + n, 2)]
            for copy in copies:
                step = max(step, ready, WRITE_FROM + sent // 8 - 1)
                sent += 4 if n == 1 else 1
                plan.setdefault(min(step, nb * spb - 1), []).append(copy)
            first += n
        assert first == spb
    return plan


def _kernel(x_hbm, w_hbm, b_hbm, o_hbm,
            xbuf, obuf, wbuf, bbuf, lhs, lhs_diag, bias, xsem, wsem, osem):
    NB, NK, _, _, S = x_hbm.shape
    D, F = w_hbm.shape
    H = F // 2
    SPB = S // CH
    ALL = slice(None)

    def steps(first, n):
        return pl.ds(first * CH, n * CH)

    def xstart(sem, *idx, priority=0):
        pltpu.make_async_copy(x_hbm.at[idx], xbuf.at[idx], xsem.at[sem]).start(priority=priority)

    def xwait(sem, *idx):
        pltpu.make_async_copy(xbuf.at[idx], xbuf.at[idx], xsem.at[sem]).wait()

    def ring(bi):
        return jnp.where(bi >= RING, bi - RING, bi)

    def ostart(bi, phase, first, n):
        idx = (ALL, ALL if phase is None else phase, ALL, steps(first, n))
        pltpu.make_async_copy(
            obuf.at[(ring(bi),) + idx], o_hbm.at[(bi,) + idx], osem.at[ring(bi)]).start()

    def owait(slot):
        pltpu.make_async_copy(obuf.at[slot], obuf.at[slot], osem.at[slot]).wait()

    def wcopy(i, first, n):
        rows = pl.ds(first, n)
        return pltpu.make_async_copy(w_hbm.at[rows], wbuf.at[rows], wsem.at[i])

    bcopy = pltpu.make_async_copy(b_hbm, bbuf, wsem.at[5])
    bcopy.start()
    wcopy(4, 512, KB).start()

    @pl.loop(0, 4)
    def _(i):
        j = (i & 1) * 2 + (i >> 1)
        wcopy(j, pl.multiple_of(128 * j, 128), 128).start()

    xstart(3, 0, ALL, ALL, ALL, steps(0, 2))
    xstart(4, 0, ALL, ALL, ALL, steps(2, 2))
    for p in range(4):
        xstart(0, 0, ALL, p, ALL, steps(GROUP, GROUP), priority=1)
    for p in range(4):
        xstart(1, 0, ALL, p, ALL, steps(UNIT, UNIT), priority=1)
    bg = PACED // SPB

    @pl.loop(0, 8)
    def _(p):
        for cond, b0 in ((p >= PACED_EXTRA, bg), (p < PACED_EXTRA, bg + 1)):
            pl.when(cond)(
                lambda: xstart(2, pl.ds(b0, NB - b0), ALL, p, ALL, steps(0, UNIT), priority=1))
        xstart(2, pl.ds(bg, NB - bg), ALL, p, ALL, steps(UNIT, UNIT), priority=1)

    bcopy.wait()
    bias[...] = jnp.broadcast_to(bbuf[...].reshape(1, F).astype(jnp.float32), (128, F)).T
    wt = {}
    for i in (4, 0, 2, 1, 3):
        n = min(128, D - 128 * i)
        wcopy(i, 128 * i, n).wait()
        wp = _prune(wbuf[pl.ds(128 * i, n), :])
        wt[i] = jnp.concatenate([wp] * (128 // n), axis=0).T.astype(jnp.float32)
    left = _left_operands(wt)
    for i, p in enumerate(PASSES):
        lhs[i] = pltpu.bitcast(left[p].astype(jnp.bfloat16), jnp.int32)
    for k, n in enumerate(DIAG):
        la, lb = left[n + "a"], left[n + "b"]
        for i, m in enumerate(_strassen_left(la[:H // 2], lb[:H // 2], la[H // 2:], lb[H // 2:])):
            lhs_diag[7 * k + i] = pltpu.bitcast(m.astype(jnp.bfloat16), jnp.int32)

    def dot(left_words, right):
        return jnp.dot(pltpu.bitcast(left_words, jnp.bfloat16), right.astype(jnp.bfloat16),
                       preferred_element_type=jnp.float32)

    def right_operand(bi, step, product):
        def halves(k):
            v = xbuf[bi, k, :, :, steps(step, 1)].astype(jnp.float32).reshape(KB, CH)
            return v[:, :128], v[:, 128:]

        n, i = product
        if n == 8:
            return halves(8)[i]
        (b11, b12), (b21, b22) = halves(n), halves(4 + n)
        if T_SCALE[n] != 1.0:
            b12, b22 = b12 * (1 / T_SCALE[n]), b22 * (1 / T_SCALE[n])
        return _strassen_right(b11, b12, b21, b22)[i]

    plan = _write_plan(NB, SPB)
    span = UNROLL * SPB

    def start_writes(t, step):
        runs = [[(b - 2 * UNROLL * it, *rest) for b, *rest in plan.get(it * span + step, ())]
                for it in range(NB // UNROLL)]
        lo = 0
        for hi, run in enumerate(runs):
            if hi + 1 < len(runs) and runs[hi + 1] == run:
                continue
            if run:
                @pl.when((t >= lo) & (t <= hi))
                def _():
                    for db, *rest in run:
                        ostart(2 * UNROLL * t + db, *rest)
            lo = hi + 1

    def group(t, u, g):
        bi = t * UNROLL + u
        here = bi * SPB + g
        top = u == 0 and g == 0
        if top:
            pl.when(t == 0)(lambda: xwait(3, 0, ALL, ALL, ALL, steps(0, 2)))
        if u == 0 and g == GROUP:
            pl.when(t == 0)(lambda: xwait(0, 0, ALL, ALL, ALL, steps(GROUP, GROUP)))
        if g % UNIT == 0:
            pl.when((here > 0) & (here < PACED))(
                lambda: xwait(g // UNIT, bi, ALL, ALL, ALL, steps(g, UNIT)))
            if u * SPB + g == PACED % span:
                pl.when(here == PACED)(lambda: xwait(2, pl.ds(bg, NB - bg)))
            ahead = [(g + UNIT, p) for p in range(2, 6)]
        else:
            ahead = [(g + GROUP, 6), (g + GROUP, 7), (g + GROUP + UNIT, 0), (g + GROUP + UNIT, 1)]
        if g == 0:
            pl.when(bi >= RING)(lambda: owait(bi - RING))
        todo = [(c, p, k) for c, p in ahead for k in range(NK)]
        rows_done, total = [0], len(todo)

        def fetch(rows):
            rows_done[0] += rows
            while (total - len(todo)) * (3 * GROUP * H + 7 * H // 2) < rows_done[0] * total:
                i = total - len(todo)
                c, p, k = todo.pop(0)
                step = bi * SPB + c
                wanted = step < PACED + (p < PACED_EXTRA)
                if top and p < 4:
                    wanted = wanted & (t > 0)
                    if i % 3 != 2:
                        q = i - i // 3
                        pl.when(t == 0)(lambda: xstart(
                            0, 0, pl.ds(q % 3 * 3, 3), 4 + q // 3, ALL, steps(GROUP, GROUP)))
                pl.when(wanted)(lambda: xstart(
                    jnp.where(step < PACED, c // UNIT % 2, 2),
                    bi + c // SPB, k, p, ALL, steps(c % SPB, UNIT)))

        def right_tiles(rows, build):
            half = {}
            for h in (1, 0):
                fetch(rows // 2)
                half[h] = build(h)
            return [jnp.concatenate(pair, axis=0) for pair in zip(half[0], half[1])]

        def passes(e, *names):
            right = right_tiles(
                H, lambda h: [right_operand(bi, g + e, PRODUCTS[p][h]) for p in names])
            return [dot(lhs[PASSES.index(p)], r) for p, r in zip(names, right)]

        last_passes = {0: passes(0, "p1", "pr", "q1", "qr")} if top else {}
        diag = {}
        for e in range(0, GROUP, 2):
            if top and e == 2:
                pl.when(t == 0)(lambda: xwait(4, 0, ALL, ALL, ALL, steps(2, 2)))
            for k, n in enumerate(DIAG):
                right = right_tiles(7 * H // 8, lambda h: _strassen_right(*[
                    right_operand(bi, g + e + d, PRODUCTS[n + ab][h]) for ab in "ab" for d in (0, 1)]))
                m = {i: dot(lhs_diag[7 * k + i], right[i]) for i in (0, 3, 4, 6, 2, 1, 5)}
                diag[n, e] = jnp.concatenate([(m[0] + m[3]) + (m[6] - m[4]), m[1] + m[3]], axis=0)
                diag[n, e + 1] = jnp.concatenate([m[2] + m[4], (m[0] - m[1]) + (m[2] + m[5])], axis=0)

        for e in range(GROUP):
            m1q, mrq, miq, phi = passes(e, "1Q", "rQ", "iQ", "phi")
            c11 = (m1q + mrq) + (miq + phi) + diag["n11", e]
            c21 = m1q + mrq * RHO + miq * (1 / RHO)
            c22 = diag["n22", e] + phi
            m1p, mrp, mip, psi = passes(e, "1P", "rP", "iP", "psi")
            c12 = m1p + mrp + mip
            c22 = (c22 + m1p) + (mrp + psi) * RHO + mip * (1 / RHO)
            mp1, mpr, mq1, mqr = last_passes.get(e) or passes(e, "p1", "pr", "q1", "qr")
            b1, b2 = bias[0:H], bias[H:F]
            c12 = (c12 + b1) + mp1 + mpr * RHO
            c11 = ((c11 + psi) + b1) - (mp1 + mpr)
            c21 = (c21 + b2) + (mq1 + mqr)
            c22 = (c22 + b2) - (mq1 + mqr * RHO)
            for r0, quadrants in ((0, (c11, c12)), (H, (c21, c22))):
                val = jnp.concatenate(quadrants, axis=1)
                for k in range(r0 // KB, (r0 + H - 1) // KB + 1):
                    lo, hi = max(r0, KB * k), min(r0 + H, KB * (k + 1))
                    part = val[lo - r0:hi - r0].reshape((hi - lo) // 8, 8, CH)
                    phases = pl.ds(lo % KB // 8, (hi - lo) // 8)
                    obuf[ring(bi), k, phases, :, steps(g + e, 1)] = part.astype(obuf.dtype)
            start_writes(t, u * SPB + g + e)
        assert not todo

    @pl.loop(0, NB // UNROLL)
    def _(t):
        for u in range(UNROLL):
            for g in range(0, SPB, GROUP):
                group(t, u, g)

    for bi in range(NB - RING, NB):
        owait(bi % RING)


@jax.jit
def pallas_standalone__structured_sparse_n_m__ragged_kernel(
    x: jax.Array,
    w: jax.Array,
    b: jax.Array,
):
    B, S, D = x.shape
    F = w.shape[1]
    out = pl.pallas_call(
        _kernel,
        in_specs=[pl.BlockSpec(memory_space=pl.ANY)] * 3,
        out_specs=pl.BlockSpec(memory_space=pl.ANY),
        out_shape=jax.ShapeDtypeStruct((B, F // KB, 8, 8, S), x.dtype),
        scratch_shapes=[
            pltpu.VMEM((B, D // KB, 8, 8, S), x.dtype),
            pltpu.VMEM((RING, F // KB, 8, 8, S), x.dtype),
            pltpu.VMEM((D, F), w.dtype),
            pltpu.VMEM((F,), b.dtype),
            pltpu.VMEM((len(PASSES), F // 4, 128), jnp.int32),
            pltpu.VMEM((7 * len(DIAG), F // 8, 128), jnp.int32),
            pltpu.VMEM((F, 128), jnp.float32),
            pltpu.SemaphoreType.DMA((5,)),
            pltpu.SemaphoreType.DMA((6,)),
            pltpu.SemaphoreType.DMA((RING,)),
        ],
        compiler_params=pltpu.CompilerParams(
            vmem_limit_bytes=126 * 1024 * 1024,
            disable_bounds_checks=True,
            disable_semaphore_checks=True,
            flags={"XLA_TPU_RESCHEDULE_DMA_DONES": True, "XLA_TPU_MAX_INSTS_TO_PREDICATE": 65536},
        ),
    )(jnp.transpose(x, (0, 2, 1)).reshape(B, D // KB, 8, 8, S), w, b)
    return jnp.transpose(out.reshape(B, F, S), (0, 2, 1))
```

```python
import jax
import jax.numpy as jnp
from jax import lax
import jax.experimental.pallas as pl
import jax.experimental.pallas.tpu as pltpu

KB = 64
CH = 256
GROUP = 4
UNIT = 8
UNROLL = 2

RHO = 2.0
T_SCALE = (1.0, 1.0, RHO, RHO)
PASSES = ("1Q", "rQ", "iQ", "phi", "1P", "rP", "iP", "psi", "p1", "pr", "q1", "qr")
DIAG = ("n11", "n22")
PRODUCTS = {
    "phi": ((0, 0), (3, 0)), "psi": ((2, 0), (1, 0)),
    "q1": ((0, 1), (1, 1)), "qr": ((2, 1), (3, 1)),
    "1P": ((0, 2), (2, 2)), "rP": ((8, 1), (1, 2)), "iP": ((8, 1), (3, 2)),
    "1Q": ((0, 3), (2, 3)), "rQ": ((8, 0), (1, 3)), "iQ": ((8, 0), (3, 3)),
    "p1": ((0, 4), (1, 4)), "pr": ((2, 4), (3, 4)),
    "n22a": ((0, 5), (1, 5)), "n22b": ((2, 5), (3, 5)),
    "n11a": ((0, 6), (1, 6)), "n11b": ((2, 6), (3, 6)),
}

PACED = 128
PACED_EXTRA = 4
WRITE_FROM = 122
WRITE_TAIL = {14: (14, 2), 15: (6, 4, 2, 1, 1, 1, 1)}
RING = 9


def _prune_packed(u):
    mate = lax.broadcasted_iota(jnp.int32, u.shape, 0) ^ 1
    lo = pltpu.bitcast((u << 16) & 0x7FFFFFFF, jnp.float32)
    hi = pltpu.bitcast(u & 0x7FFF0000, jnp.float32)
    big, small = jnp.maximum(lo, hi), jnp.minimum(lo, hi)
    nbig = jnp.take_along_axis(big, mate, axis=0, mode="promise_in_bounds")
    nsmall = jnp.take_along_axis(small, mate, axis=0, mode="promise_in_bounds")
    thr = jnp.maximum(jnp.minimum(big, nbig), jnp.maximum(small, nsmall))
    return u & (jnp.where(lo < thr, 0, 0xFFFF) | jnp.where(hi < thr, 0, -65536))


def _prune(w):
    u = pltpu.bitcast(w, jnp.int32)
    parts = [_prune_packed(u[8 * i:8 * i + 8]) for i in range(u.shape[0] // 8)]
    return pltpu.bitcast(jnp.concatenate(parts, axis=0), jnp.bfloat16)


def _strassen_left(a11, a12, a21, a22):
    return [a11 + a22, a21 + a22, a11, a22, a11 + a12, a21 - a11, a12 - a22]


def _strassen_right(b11, b12, b21, b22):
    return [b11 - b22, b11, b12 - b22, b21 - b11, b22, b11 - b12, b21 - b22]


def _left_operands(wt):
    h = wt[0].shape[0] // 2
    low = lax.broadcasted_iota(jnp.int32, (h, 128), 1) < KB
    mix = lambda a, b: jnp.where(low, a, b)
    per_block = lambda a, b: jnp.where(low[0:1], a, b)
    inv_ab, inv_cd = per_block(1.0, 1 / RHO), per_block(1.0, RHO)
    ab = _strassen_left(wt[0][:h], wt[2][:h], wt[0][h:] * inv_ab, wt[2][h:] * inv_ab)
    cd = _strassen_left(wt[1][:h], wt[3][:h], wt[1][h:] * inv_cd, wt[3][h:] * inv_cd)
    u = (wt[4][h:] - wt[4][:h] * (1 / RHO)) * (1 / (RHO - 1 / RHO))
    v = (wt[4][:h] * RHO - wt[4][h:]) * (1 / (RHO - 1 / RHO))
    cd2 = cd[2] * RHO
    return {
        "phi": mix(ab[0], cd[0]), "psi": mix(cd[0], ab[0]),
        "q1": ab[1] * per_block(1.0, RHO), "qr": cd[1] * per_block(1.0, 1 / RHO),
        "1P": mix(ab[2], pltpu.roll(cd2, KB, 1)), "rP": mix(u, ab[2]), "iP": mix(v, cd2),
        "1Q": mix(ab[3], pltpu.roll(cd[3], KB, 1)), "rQ": mix(u, ab[3]), "iQ": mix(v, cd[3]),
        "p1": ab[4], "pr": cd[4],
        "n22a": ab[5] * per_block(1.0, RHO), "n22b": cd[5] * per_block(RHO, 1.0),
        "n11a": ab[6], "n11b": cd[6],
    }


def _write_plan(nb, spb):
    plan, step, sent = {}, WRITE_FROM, 0
    for b in range(nb):
        first = 0
        for n in WRITE_TAIL.get(b, (spb,)):
            ready = b * spb + first + n - 1
            if n == 1:
                copies = [(b, None, first, 1)]
            else:
                copies = [(b, p, c, 2) for p in range(8) for c in range(first, first + n, 2)]
            for copy in copies:
                step = max(step, ready, WRITE_FROM + sent // 8 - 1)
                sent += 4 if n == 1 else 1
                plan.setdefault(min(step, nb * spb - 1), []).append(copy)
            first += n
        assert first == spb
    return plan


def _kernel(x_hbm, w_hbm, b_hbm, o_hbm,
            xbuf, obuf, wbuf, bbuf, lhs, lhs_diag, bias, xsem, wsem, osem):
    NB, NK, _, _, S = x_hbm.shape
    D, F = w_hbm.shape
    H = F // 2
    SPB = S // CH
    ALL = slice(None)

    def steps(first, n):
        return pl.ds(first * CH, n * CH)

    def xstart(sem, *idx, priority=0):
        pltpu.make_async_copy(x_hbm.at[idx], xbuf.at[idx], xsem.at[sem]).start(priority=priority)

    def xwait(sem, *idx):
        pltpu.make_async_copy(xbuf.at[idx], xbuf.at[idx], xsem.at[sem]).wait()

    def ring(bi):
        return jnp.where(bi >= RING, bi - RING, bi)

    def ostart(bi, phase, first, n):
        idx = (ALL, ALL if phase is None else phase, ALL, steps(first, n))
        pltpu.make_async_copy(
            obuf.at[(ring(bi),) + idx], o_hbm.at[(bi,) + idx], osem.at[ring(bi)]).start()

    def owait(slot):
        pltpu.make_async_copy(obuf.at[slot], obuf.at[slot], osem.at[slot]).wait()

    def wcopy(i, first, n):
        rows = pl.ds(first, n)
        return pltpu.make_async_copy(w_hbm.at[rows], wbuf.at[rows], wsem.at[i])

    bcopy = pltpu.make_async_copy(b_hbm, bbuf, wsem.at[5])
    bcopy.start()
    wcopy(4, 512, KB).start()

    @pl.loop(0, 4)
    def _(i):
        j = (i & 1) * 2 + (i >> 1)
        wcopy(j, pl.multiple_of(128 * j, 128), 128).start()

    xstart(3, 0, ALL, ALL, ALL, steps(0, GROUP))
    for p in range(4):
        xstart(0, 0, ALL, p, ALL, steps(GROUP, GROUP), priority=1)
    for p in range(4):
        xstart(1, 0, ALL, p, ALL, steps(UNIT, UNIT), priority=1)
    bg = PACED // SPB

    @pl.loop(0, 8)
    def _(p):
        for cond, b0 in ((p >= PACED_EXTRA, bg), (p < PACED_EXTRA, bg + 1)):
            pl.when(cond)(
                lambda: xstart(2, pl.ds(b0, NB - b0), ALL, p, ALL, steps(0, UNIT), priority=1))
        xstart(2, pl.ds(bg, NB - bg), ALL, p, ALL, steps(UNIT, UNIT), priority=1)

    bcopy.wait()
    bias[...] = jnp.broadcast_to(bbuf[...].reshape(1, F).astype(jnp.float32), (128, F)).T
    wt = {}
    for i in (4, 0, 2, 1, 3):
        n = min(128, D - 128 * i)
        wcopy(i, 128 * i, n).wait()
        wp = _prune(wbuf[pl.ds(128 * i, n), :])
        wt[i] = jnp.concatenate([wp] * (128 // n), axis=0).T.astype(jnp.float32)
    left = _left_operands(wt)
    for i, p in enumerate(PASSES):
        lhs[i] = pltpu.bitcast(left[p].astype(jnp.bfloat16), jnp.int32)
    for k, n in enumerate(DIAG):
        la, lb = left[n + "a"], left[n + "b"]
        for i, m in enumerate(_strassen_left(la[:H // 2], lb[:H // 2], la[H // 2:], lb[H // 2:])):
            lhs_diag[7 * k + i] = pltpu.bitcast(m.astype(jnp.bfloat16), jnp.int32)

    def dot(left_words, right):
        return jnp.dot(pltpu.bitcast(left_words, jnp.bfloat16), right.astype(jnp.bfloat16),
                       preferred_element_type=jnp.float32)

    def right_operand(bi, step, product):
        def halves(k):
            v = xbuf[bi, k, :, :, steps(step, 1)].astype(jnp.float32).reshape(KB, CH)
            return v[:, :128], v[:, 128:]

        n, i = product
        if n == 8:
            return halves(8)[i]
        (b11, b12), (b21, b22) = halves(n), halves(4 + n)
        if T_SCALE[n] != 1.0:
            b12, b22 = b12 * (1 / T_SCALE[n]), b22 * (1 / T_SCALE[n])
        return _strassen_right(b11, b12, b21, b22)[i]

    plan = _write_plan(NB, SPB)
    span = UNROLL * SPB

    def start_writes(t, step):
        runs = [[(b - 2 * UNROLL * it, *rest) for b, *rest in plan.get(it * span + step, ())]
                for it in range(NB // UNROLL)]
        lo = 0
        for hi, run in enumerate(runs):
            if hi + 1 < len(runs) and runs[hi + 1] == run:
                continue
            if run:
                @pl.when((t >= lo) & (t <= hi))
                def _():
                    for db, *rest in run:
                        ostart(2 * UNROLL * t + db, *rest)
            lo = hi + 1

    def group(t, u, g):
        bi = t * UNROLL + u
        here = bi * SPB + g
        top = u == 0 and g == 0
        if top:
            pl.when(t == 0)(lambda: xwait(3, 0, ALL, ALL, ALL, steps(0, GROUP)))
        if u == 0 and g == GROUP:
            pl.when(t == 0)(lambda: xwait(0, 0, ALL, ALL, ALL, steps(GROUP, GROUP)))
        if g % UNIT == 0:
            pl.when((here > 0) & (here < PACED))(
                lambda: xwait(g // UNIT, bi, ALL, ALL, ALL, steps(g, UNIT)))
            if u * SPB + g == PACED % span:
                pl.when(here == PACED)(lambda: xwait(2, pl.ds(bg, NB - bg)))
            ahead = [(g + UNIT, p) for p in range(2, 6)]
        else:
            ahead = [(g + GROUP, 6), (g + GROUP, 7), (g + GROUP + UNIT, 0), (g + GROUP + UNIT, 1)]
        if g == 0:
            pl.when(bi >= RING)(lambda: owait(bi - RING))
        todo = [(c, p, k) for c, p in ahead for k in range(NK)]
        rows_done, total = [0], len(todo)

        def fetch(rows):
            rows_done[0] += rows
            while (total - len(todo)) * (3 * GROUP * H + 7 * H // 2) < rows_done[0] * total:
                i = total - len(todo)
                c, p, k = todo.pop(0)
                step = bi * SPB + c
                wanted = step < PACED + (p < PACED_EXTRA)
                if top and p < 4:
                    wanted = wanted & (t > 0)
                    if i % 3 != 2:
                        q = i - i // 3
                        pl.when(t == 0)(lambda: xstart(
                            0, 0, pl.ds(q % 3 * 3, 3), 4 + q // 3, ALL, steps(GROUP, GROUP)))
                pl.when(wanted)(lambda: xstart(
                    jnp.where(step < PACED, c // UNIT % 2, 2),
                    bi + c // SPB, k, p, ALL, steps(c % SPB, UNIT)))

        def right_tiles(rows, build):
            half = {}
            for h in (1, 0):
                fetch(rows // 2)
                half[h] = build(h)
            return [jnp.concatenate(pair, axis=0) for pair in zip(half[0], half[1])]

        def passes(e, *names):
            right = right_tiles(
                H, lambda h: [right_operand(bi, g + e, PRODUCTS[p][h]) for p in names])
            return [dot(lhs[PASSES.index(p)], r) for p, r in zip(names, right)]

        last_passes = {0: passes(0, "p1", "pr", "q1", "qr")} if top else {}
        diag = {}
        for e in range(0, GROUP, 2):
            for k, n in enumerate(DIAG):
                right = right_tiles(7 * H // 8, lambda h: _strassen_right(*[
                    right_operand(bi, g + e + d, PRODUCTS[n + ab][h]) for ab in "ab" for d in (0, 1)]))
                m = {i: dot(lhs_diag[7 * k + i], right[i]) for i in (0, 3, 4, 6, 2, 1, 5)}
                diag[n, e] = jnp.concatenate([(m[0] + m[3]) + (m[4] + m[6]), m[1] + m[3]], axis=0)
                diag[n, e + 1] = jnp.concatenate([m[2] + m[4], (m[1] - m[0]) + (m[2] - m[5])], axis=0)

        for e in range(GROUP):
            m1q, mrq, miq, phi = passes(e, "1Q", "rQ", "iQ", "phi")
            c11 = (m1q + mrq) + (miq + phi) + diag["n11", e]
            c21 = m1q + mrq * RHO + miq * (1 / RHO)
            minus_c22 = diag["n22", e] + phi
            m1p, mrp, mip, psi = passes(e, "1P", "rP", "iP", "psi")
            c12 = m1p + mrp + mip
            c22 = (m1p - minus_c22) + (mrp - psi) * RHO + mip * (1 / RHO)
            mp1, mpr, mq1, mqr = last_passes.get(e) or passes(e, "p1", "pr", "q1", "qr")
            b1, b2 = bias[0:H], bias[H:F]
            c12 = (c12 + b1) + mp1 + mpr * RHO
            c11 = ((c11 + psi) + b1) + (mp1 + mpr)
            c21 = (c21 + b2) + (mq1 + mqr)
            c22 = (c22 + b2) + (mq1 + mqr * RHO)
            for r0, quadrants in ((0, (c11, c12)), (H, (c21, c22))):
                val = jnp.concatenate(quadrants, axis=1)
                for k in range(r0 // KB, (r0 + H - 1) // KB + 1):
                    lo, hi = max(r0, KB * k), min(r0 + H, KB * (k + 1))
                    part = val[lo - r0:hi - r0].reshape((hi - lo) // 8, 8, CH)
                    phases = pl.ds(lo % KB // 8, (hi - lo) // 8)
                    obuf[ring(bi), k, phases, :, steps(g + e, 1)] = part.astype(obuf.dtype)
            start_writes(t, u * SPB + g + e)
        assert not todo

    @pl.loop(0, NB // UNROLL)
    def _(t):
        for u in range(UNROLL):
            for g in range(0, SPB, GROUP):
                group(t, u, g)

    for bi in range(NB - RING, NB):
        owait(bi % RING)


@jax.jit
def pallas_standalone__structured_sparse_n_m__ragged_kernel(
    x: jax.Array,
    w: jax.Array,
    b: jax.Array,
):
    B, S, D = x.shape
    F = w.shape[1]
    out = pl.pallas_call(
        _kernel,
        in_specs=[pl.BlockSpec(memory_space=pl.ANY)] * 3,
        out_specs=pl.BlockSpec(memory_space=pl.ANY),
        out_shape=jax.ShapeDtypeStruct((B, F // KB, 8, 8, S), x.dtype),
        scratch_shapes=[
            pltpu.VMEM((B, D // KB, 8, 8, S), x.dtype),
            pltpu.VMEM((RING, F // KB, 8, 8, S), x.dtype),
            pltpu.VMEM((D, F), w.dtype),
            pltpu.VMEM((F,), b.dtype),
            pltpu.VMEM((len(PASSES), F // 4, 128), jnp.int32),
            pltpu.VMEM((7 * len(DIAG), F // 8, 128), jnp.int32),
            pltpu.VMEM((F, 128), jnp.float32),
            pltpu.SemaphoreType.DMA((4,)),
            pltpu.SemaphoreType.DMA((6,)),
            pltpu.SemaphoreType.DMA((RING,)),
        ],
        compiler_params=pltpu.CompilerParams(
            vmem_limit_bytes=126 * 1024 * 1024,
            disable_bounds_checks=True,
            disable_semaphore_checks=True,
            flags={"XLA_TPU_RESCHEDULE_DMA_DONES": True, "XLA_TPU_MAX_INSTS_TO_PREDICATE": 65536},
        ),
    )(jnp.transpose(x, (0, 2, 1)).reshape(B, D // KB, 8, 8, S), w, b)
    return jnp.transpose(out.reshape(B, F, S), (0, 2, 1))
```

```python
import jax
import jax.numpy as jnp
from jax import lax
import jax.experimental.pallas as pl
import jax.experimental.pallas.tpu as pltpu

KB = 64
CH = 256
GROUP = 4
UNIT = 8
UNROLL = 2

RHO = 2.0
T_SCALE = (1.0, 1.0, RHO, RHO)
PASSES = ("1Q", "rQ", "iQ", "phi", "1P", "rP", "iP", "psi", "p1", "pr", "q1", "qr")
DIAG = ("n11", "n22")
PRODUCTS = {
    "phi": ((0, 0), (3, 0)), "psi": ((2, 0), (1, 0)),
    "q1": ((0, 1), (1, 1)), "qr": ((2, 1), (3, 1)),
    "1P": ((0, 2), (2, 2)), "rP": ((8, 1), (1, 2)), "iP": ((8, 1), (3, 2)),
    "1Q": ((0, 3), (2, 3)), "rQ": ((8, 0), (1, 3)), "iQ": ((8, 0), (3, 3)),
    "p1": ((0, 4), (1, 4)), "pr": ((2, 4), (3, 4)),
    "n22a": ((0, 5), (1, 5)), "n22b": ((2, 5), (3, 5)),
    "n11a": ((0, 6), (1, 6)), "n11b": ((2, 6), (3, 6)),
}

PACED = 128
PACED_EXTRA = 4
WRITE_FROM = 122
WRITE_TAIL = {14: (14, 2), 15: (6, 4, 2, 1, 1, 1, 1)}
RING = 9


def _prune_packed(u):
    mate = lax.broadcasted_iota(jnp.int32, u.shape, 0) ^ 1
    lo = pltpu.bitcast((u << 16) & 0x7FFFFFFF, jnp.float32)
    hi = pltpu.bitcast(u & 0x7FFF0000, jnp.float32)
    big, small = jnp.maximum(lo, hi), jnp.minimum(lo, hi)
    nbig = jnp.take_along_axis(big, mate, axis=0, mode="promise_in_bounds")
    nsmall = jnp.take_along_axis(small, mate, axis=0, mode="promise_in_bounds")
    thr = jnp.maximum(jnp.minimum(big, nbig), jnp.maximum(small, nsmall))
    return u & (jnp.where(lo < thr, 0, 0xFFFF) | jnp.where(hi < thr, 0, -65536))


def _prune(w):
    u = pltpu.bitcast(w, jnp.int32)
    parts = [_prune_packed(u[8 * i:8 * i + 8]) for i in range(u.shape[0] // 8)]
    return pltpu.bitcast(jnp.concatenate(parts, axis=0), jnp.bfloat16)


def _strassen_left(a11, a12, a21, a22):
    return [a11 + a22, a21 + a22, a11, a22, a11 + a12, a21 - a11, a12 - a22]


def _strassen_right(b11, b12, b21, b22):
    return [b11 - b22, b11, b12 - b22, b21 - b11, b22, b11 - b12, b21 - b22]


def _equilibrate(wt):
    exponent = pltpu.bitcast(jnp.max(jnp.abs(wt), axis=0, keepdims=True), jnp.int32) >> 23
    exponent = jnp.minimum(exponent, 253)
    inverse = pltpu.bitcast((254 - exponent) << 23, jnp.float32)
    return wt * inverse, pltpu.bitcast(exponent << 23, jnp.float32)


def _left_operands(wt, d):
    h = wt[0].shape[0] // 2
    low = lax.broadcasted_iota(jnp.int32, (h, 128), 1) < KB
    mix = lambda a, b: jnp.where(low, a, b)
    per_block = lambda a, b: jnp.where(low[0:1], a, b)
    inv_ab, inv_cd = per_block(1.0, 1 / RHO), per_block(1.0, RHO)
    ab = _strassen_left(wt[0][:h], wt[2][:h], wt[0][h:] * inv_ab, wt[2][h:] * inv_ab)
    cd = _strassen_left(wt[1][:h], wt[3][:h], wt[1][h:] * inv_cd, wt[3][h:] * inv_cd)
    u = (wt[4][h:] - wt[4][:h] * (1 / RHO)) * (1 / (RHO - 1 / RHO))
    v = (wt[4][:h] * RHO - wt[4][h:]) * (1 / (RHO - 1 / RHO))
    cd2 = cd[2] * RHO
    return {
        "phi": mix(ab[0], cd[0]), "psi": mix(cd[0], ab[0]),
        "q1": ab[1] * (d[0] * per_block(1.0, RHO)), "qr": cd[1] * (d[1] * per_block(1.0, 1 / RHO)),
        "1P": mix(ab[2], pltpu.roll(cd2, KB, 1)), "rP": mix(u, ab[2]), "iP": mix(v, cd2),
        "1Q": mix(ab[3], pltpu.roll(cd[3], KB, 1)), "rQ": mix(u, ab[3]), "iQ": mix(v, cd[3]),
        "p1": ab[4] * d[2], "pr": cd[4] * (d[3] * (1 / RHO)),
        "n22a": ab[5] * per_block(1.0, RHO), "n22b": cd[5] * per_block(RHO, 1.0),
        "n11a": ab[6], "n11b": cd[6],
    }


def _write_plan(nb, spb):
    plan, step, sent = {}, WRITE_FROM, 0
    for b in range(nb):
        first = 0
        for n in WRITE_TAIL.get(b, (spb,)):
            ready = b * spb + first + n - 1
            if n == 1:
                copies = [(b, None, first, 1)]
            else:
                copies = [(b, p, c, 2) for p in range(8) for c in range(first, first + n, 2)]
            for copy in copies:
                step = max(step, ready, WRITE_FROM + sent // 8 - 1)
                sent += 4 if n == 1 else 1
                plan.setdefault(min(step, nb * spb - 1), []).append(copy)
            first += n
        assert first == spb
    return plan


def _kernel(x_hbm, w_hbm, b_hbm, o_hbm,
            xbuf, obuf, wbuf, bbuf, lhs, lhs_diag, bias, xscale, xsem, wsem, osem):
    NB, NK, _, _, S = x_hbm.shape
    D, F = w_hbm.shape
    H = F // 2
    SPB = S // CH
    ALL = slice(None)

    def steps(first, n):
        return pl.ds(first * CH, n * CH)

    def xstart(sem, *idx, priority=0):
        pltpu.make_async_copy(x_hbm.at[idx], xbuf.at[idx], xsem.at[sem]).start(priority=priority)

    def xwait(sem, *idx):
        pltpu.make_async_copy(xbuf.at[idx], xbuf.at[idx], xsem.at[sem]).wait()

    def ring(bi):
        return jnp.where(bi >= RING, bi - RING, bi)

    def ostart(bi, phase, first, n):
        idx = (ALL, ALL if phase is None else phase, ALL, steps(first, n))
        pltpu.make_async_copy(
            obuf.at[(ring(bi),) + idx], o_hbm.at[(bi,) + idx], osem.at[ring(bi)]).start()

    def owait(slot):
        pltpu.make_async_copy(obuf.at[slot], obuf.at[slot], osem.at[slot]).wait()

    def wcopy(i, first, n):
        rows = pl.ds(first, n)
        return pltpu.make_async_copy(w_hbm.at[rows], wbuf.at[rows], wsem.at[i])

    bcopy = pltpu.make_async_copy(b_hbm, bbuf, wsem.at[5])
    bcopy.start()
    wcopy(4, 512, KB).start()

    @pl.loop(0, 4)
    def _(i):
        j = (i & 1) * 2 + (i >> 1)
        wcopy(j, pl.multiple_of(128 * j, 128), 128).start()

    xstart(3, 0, ALL, ALL, ALL, steps(0, GROUP))
    for p in range(4):
        xstart(0, 0, ALL, p, ALL, steps(GROUP, GROUP), priority=1)
    for p in range(4):
        xstart(1, 0, ALL, p, ALL, steps(UNIT, UNIT), priority=1)
    bg = PACED // SPB

    @pl.loop(0, 8)
    def _(p):
        for cond, b0 in ((p >= PACED_EXTRA, bg), (p < PACED_EXTRA, bg + 1)):
            pl.when(cond)(
                lambda: xstart(2, pl.ds(b0, NB - b0), ALL, p, ALL, steps(0, UNIT), priority=1))
        xstart(2, pl.ds(bg, NB - bg), ALL, p, ALL, steps(UNIT, UNIT), priority=1)

    bcopy.wait()
    bias[...] = jnp.broadcast_to(bbuf[...].reshape(1, F).astype(jnp.float32), (128, F)).T
    wt, d = {}, {}
    for i in (4, 0, 2, 1, 3):
        n = min(128, D - 128 * i)
        wcopy(i, 128 * i, n).wait()
        wp = _prune(wbuf[pl.ds(128 * i, n), :])
        wt[i] = jnp.concatenate([wp] * (128 // n), axis=0).T.astype(jnp.float32)
        if i < 4:
            wt[i], d[i] = _equilibrate(wt[i])
            rows, column = pl.ds(128 * i, 128), jnp.broadcast_to(d[i], (128, 128)).T
            xscale[0, rows] = column
            xscale[1, rows] = column * (1 / T_SCALE[2 * i % 4])
    left = _left_operands(wt, d)
    for i, p in enumerate(PASSES):
        lhs[i] = pltpu.bitcast(left[p].astype(jnp.bfloat16), jnp.int32)
    for k, n in enumerate(DIAG):
        la, lb = left[n + "a"], left[n + "b"]
        for i, m in enumerate(_strassen_left(la[:H // 2], lb[:H // 2], la[H // 2:], lb[H // 2:])):
            lhs_diag[7 * k + i] = pltpu.bitcast(m.astype(jnp.bfloat16), jnp.int32)

    def dot(left_words, right):
        return jnp.dot(pltpu.bitcast(left_words, jnp.bfloat16), right.astype(jnp.bfloat16),
                       preferred_element_type=jnp.float32)

    def right_operand(bi, step, product):
        def halves(k):
            v = xbuf[bi, k, :, :, steps(step, 1)].astype(jnp.float32).reshape(KB, CH)
            return v[:, :128], v[:, 128:]

        def scaled(k):
            first, second = halves(k)
            rows = pl.ds(KB * k, KB)
            return first * xscale[0, rows], second * xscale[int(T_SCALE[k % 4] != 1.0), rows]

        n, i = product
        if n == 8:
            return halves(8)[i]
        if i in (1, 4):
            return halves(n)[0] if i == 1 else halves(4 + n)[1]
        return _strassen_right(*scaled(n), *scaled(4 + n))[i]

    plan = _write_plan(NB, SPB)
    span = UNROLL * SPB

    def start_writes(t, step):
        runs = [[(b - 2 * UNROLL * it, *rest) for b, *rest in plan.get(it * span + step, ())]
                for it in range(NB // UNROLL)]
        lo = 0
        for hi, run in enumerate(runs):
            if hi + 1 < len(runs) and runs[hi + 1] == run:
                continue
            if run:
                @pl.when((t >= lo) & (t <= hi))
                def _():
                    for db, *rest in run:
                        ostart(2 * UNROLL * t + db, *rest)
            lo = hi + 1

    def group(t, u, g):
        bi = t * UNROLL + u
        here = bi * SPB + g
        top = u == 0 and g == 0
        if top:
            pl.when(t == 0)(lambda: xwait(3, 0, ALL, ALL, ALL, steps(0, GROUP)))
        if u == 0 and g == GROUP:
            pl.when(t == 0)(lambda: xwait(0, 0, ALL, ALL, ALL, steps(GROUP, GROUP)))
        if g % UNIT == 0:
            pl.when((here > 0) & (here < PACED))(
                lambda: xwait(g // UNIT, bi, ALL, ALL, ALL, steps(g, UNIT)))
            if u * SPB + g == PACED % span:
                pl.when(here == PACED)(lambda: xwait(2, pl.ds(bg, NB - bg)))
            ahead = [(g + UNIT, p) for p in range(2, 6)]
        else:
            ahead = [(g + GROUP, 6), (g + GROUP, 7), (g + GROUP + UNIT, 0), (g + GROUP + UNIT, 1)]
        if g == 0:
            pl.when(bi >= RING)(lambda: owait(bi - RING))
        todo = [(c, p, k) for c, p in ahead for k in range(NK)]
        rows_done, total = [0], len(todo)

        def fetch(rows):
            rows_done[0] += rows
            while (total - len(todo)) * (3 * GROUP * H + 7 * H // 2) < rows_done[0] * total:
                i = total - len(todo)
                c, p, k = todo.pop(0)
                step = bi * SPB + c
                wanted = step < PACED + (p < PACED_EXTRA)
                if top and p < 4:
                    wanted = wanted & (t > 0)
                    if i % 3 != 2:
                        q = i - i // 3
                        pl.when(t == 0)(lambda: xstart(
                            0, 0, pl.ds(q % 3 * 3, 3), 4 + q // 3, ALL, steps(GROUP, GROUP)))
                pl.when(wanted)(lambda: xstart(
                    jnp.where(step < PACED, c // UNIT % 2, 2),
                    bi + c // SPB, k, p, ALL, steps(c % SPB, UNIT)))

        def right_tiles(rows, build):
            half = {}
            for h in (1, 0):
                fetch(rows // 2)
                half[h] = build(h)
            return [jnp.concatenate(pair, axis=0) for pair in zip(half[0], half[1])]

        def passes(e, *names):
            right = right_tiles(
                H, lambda h: [right_operand(bi, g + e, PRODUCTS[p][h]) for p in names])
            return [dot(lhs[PASSES.index(p)], r) for p, r in zip(names, right)]

        last_passes = {0: passes(0, "p1", "pr", "q1", "qr")} if top else {}
        diag = {}
        for e in range(0, GROUP, 2):
            for k, n in enumerate(DIAG):
                right = right_tiles(7 * H // 8, lambda h: _strassen_right(*[
                    right_operand(bi, g + e + d, PRODUCTS[n + ab][h]) for ab in "ab" for d in (0, 1)]))
                m = {i: dot(lhs_diag[7 * k + i], right[i]) for i in (0, 3, 4, 6, 2, 1, 5)}
                diag[n, e] = jnp.concatenate([(m[0] + m[3]) + (m[4] + m[6]), m[1] + m[3]], axis=0)
                diag[n, e + 1] = jnp.concatenate([m[2] + m[4], (m[1] - m[0]) + (m[2] - m[5])], axis=0)

        for e in range(GROUP):
            m1q, mrq, miq, phi = passes(e, "1Q", "rQ", "iQ", "phi")
            c11 = (m1q + mrq) + (miq + phi) + diag["n11", e]
            c21 = m1q + mrq * RHO + miq * (1 / RHO)
            minus_c22 = diag["n22", e] + phi
            m1p, mrp, mip, psi = passes(e, "1P", "rP", "iP", "psi")
            c12 = m1p + mrp + mip
            c22 = (m1p - minus_c22) + (mrp - psi) * RHO + mip * (1 / RHO)
            mp1, mpr, mq1, mqr = last_passes.get(e) or passes(e, "p1", "pr", "q1", "qr")
            b1, b2 = bias[0:H], bias[H:F]
            c12 = (c12 + b1) + mp1 + mpr * RHO
            c11 = ((c11 + psi) + b1) + (mp1 + mpr)
            c21 = (c21 + b2) + (mq1 + mqr)
            c22 = (c22 + b2) + (mq1 + mqr * RHO)
            for r0, quadrants in ((0, (c11, c12)), (H, (c21, c22))):
                val = jnp.concatenate(quadrants, axis=1)
                for k in range(r0 // KB, (r0 + H - 1) // KB + 1):
                    lo, hi = max(r0, KB * k), min(r0 + H, KB * (k + 1))
                    part = val[lo - r0:hi - r0].reshape((hi - lo) // 8, 8, CH)
                    phases = pl.ds(lo % KB // 8, (hi - lo) // 8)
                    obuf[ring(bi), k, phases, :, steps(g + e, 1)] = part.astype(obuf.dtype)
            start_writes(t, u * SPB + g + e)
        assert not todo

    @pl.loop(0, NB // UNROLL)
    def _(t):
        for u in range(UNROLL):
            for g in range(0, SPB, GROUP):
                group(t, u, g)

    for bi in range(NB - RING, NB):
        owait(bi % RING)


@jax.jit
def pallas_standalone__structured_sparse_n_m__ragged_kernel(
    x: jax.Array,
    w: jax.Array,
    b: jax.Array,
):
    B, S, D = x.shape
    F = w.shape[1]
    out = pl.pallas_call(
        _kernel,
        in_specs=[pl.BlockSpec(memory_space=pl.ANY)] * 3,
        out_specs=pl.BlockSpec(memory_space=pl.ANY),
        out_shape=jax.ShapeDtypeStruct((B, F // KB, 8, 8, S), x.dtype),
        scratch_shapes=[
            pltpu.VMEM((B, D // KB, 8, 8, S), x.dtype),
            pltpu.VMEM((RING, F // KB, 8, 8, S), x.dtype),
            pltpu.VMEM((D, F), w.dtype),
            pltpu.VMEM((F,), b.dtype),
            pltpu.VMEM((len(PASSES), F // 4, 128), jnp.int32),
            pltpu.VMEM((7 * len(DIAG), F // 8, 128), jnp.int32),
            pltpu.VMEM((F, 128), jnp.float32),
            pltpu.VMEM((2, 8 * KB, 128), jnp.float32),
            pltpu.SemaphoreType.DMA((4,)),
            pltpu.SemaphoreType.DMA((6,)),
            pltpu.SemaphoreType.DMA((RING,)),
        ],
        compiler_params=pltpu.CompilerParams(
            vmem_limit_bytes=126 * 1024 * 1024,
            disable_bounds_checks=True,
            disable_semaphore_checks=True,
            flags={"XLA_TPU_RESCHEDULE_DMA_DONES": True, "XLA_TPU_MAX_INSTS_TO_PREDICATE": 65536},
        ),
    )(jnp.transpose(x, (0, 2, 1)).reshape(B, D // KB, 8, 8, S), w, b)
    return jnp.transpose(out.reshape(B, F, S), (0, 2, 1))
```

```python
import jax
import jax.numpy as jnp
from jax import lax
import jax.experimental.pallas as pl
import jax.experimental.pallas.tpu as pltpu

KB = 64
CH = 256
GROUP = 4
UNIT = 8
UNROLL = 2

RHO = 2.0
T_SCALE = (1.0, 1.0, RHO, RHO)
PASSES = ("1Q", "rQ", "iQ", "phi", "1P", "rP", "iP", "psi", "p1", "pr", "q1", "qr")
DIAG = ("n11", "n22")
PRODUCTS = {
    "phi": ((0, 0), (3, 0)), "psi": ((2, 0), (1, 0)),
    "q1": ((0, 1), (1, 1)), "qr": ((2, 1), (3, 1)),
    "1P": ((0, 2), (2, 2)), "rP": ((8, 1), (1, 2)), "iP": ((8, 1), (3, 2)),
    "1Q": ((0, 3), (2, 3)), "rQ": ((8, 0), (1, 3)), "iQ": ((8, 0), (3, 3)),
    "p1": ((0, 4), (1, 4)), "pr": ((2, 4), (3, 4)),
    "n22a": ((0, 5), (1, 5)), "n22b": ((2, 5), (3, 5)),
    "n11a": ((0, 6), (1, 6)), "n11b": ((2, 6), (3, 6)),
}

PACED = 128
PACED_EXTRA = 4
WRITE_FROM = 122
WRITE_TAIL = {14: (14, 2), 15: (6, 4, 2, 1, 1, 1, 1)}
RING = 9


def _prune_packed(u):
    mate = lax.broadcasted_iota(jnp.int32, u.shape, 0) ^ 1
    lo = pltpu.bitcast((u << 16) & 0x7FFFFFFF, jnp.float32)
    hi = pltpu.bitcast(u & 0x7FFF0000, jnp.float32)
    big, small = jnp.maximum(lo, hi), jnp.minimum(lo, hi)
    nbig = jnp.take_along_axis(big, mate, axis=0, mode="promise_in_bounds")
    nsmall = jnp.take_along_axis(small, mate, axis=0, mode="promise_in_bounds")
    thr = jnp.maximum(jnp.minimum(big, nbig), jnp.maximum(small, nsmall))
    return u & (jnp.where(lo < thr, 0, 0xFFFF) | jnp.where(hi < thr, 0, -65536))


def _prune(w):
    u = pltpu.bitcast(w, jnp.int32)
    parts = [_prune_packed(u[8 * i:8 * i + 8]) for i in range(u.shape[0] // 8)]
    return pltpu.bitcast(jnp.concatenate(parts, axis=0), jnp.bfloat16)


def _strassen_left(a11, a12, a21, a22):
    return [a11 + a22, a21 + a22, a11, a22, a11 + a12, a21 - a11, a12 - a22]


def _strassen_right(b11, b12, b21, b22):
    return [b11 - b22, b11, b12 - b22, b21 - b11, b22, b11 - b12, b21 - b22]


def _to_words(v):
    return pltpu.bitcast(v.astype(jnp.bfloat16), jnp.int32)


def _from_words(u):
    return pltpu.bitcast(u, jnp.bfloat16)


def _row_scale(wt):
    largest = jnp.max(jnp.abs(wt.astype(jnp.float32)), axis=0, keepdims=True)
    exponent = jnp.clip(pltpu.bitcast(largest, jnp.int32) >> 23, 2, 252)
    d = pltpu.bitcast(exponent << 23, jnp.float32)
    return jnp.where(largest == 0.0, 0.0, d), pltpu.bitcast((254 - exponent) << 23, jnp.float32)


def _left_operands(upper, lower, d, inv_d):
    low = lax.broadcasted_iota(jnp.int32, upper[0].shape, 1) < KB
    mix = lambda a, b: jnp.where(low, a, b)
    per_block = lambda a, b: jnp.where(low[0:1], a, b)
    ab, cd = [
        _strassen_left(upper[i] * inv_d[i], upper[i + 2] * inv_d[i + 2],
                       lower[i] * (inv_d[i] * inv_s), lower[i + 2] * (inv_d[i + 2] * inv_s))
        for i, inv_s in enumerate((per_block(1.0, 1 / RHO), per_block(1.0, RHO)))]
    u = (lower[4] - upper[4] * (1 / RHO)) * (1 / (RHO - 1 / RHO))
    v = (upper[4] * RHO - lower[4]) * (1 / (RHO - 1 / RHO))
    return {
        "phi": mix(ab[0], cd[0]), "psi": mix(cd[0], ab[0]),
        "q1": ab[1] * (d[0] * per_block(1.0, RHO)), "qr": cd[1] * (d[1] * per_block(1.0, 1 / RHO)),
        "1P": mix(ab[2], pltpu.roll(cd[2], KB, 1)), "rP": mix(u, ab[2]), "iP": mix(v, cd[2]),
        "1Q": mix(ab[3], pltpu.roll(cd[3], KB, 1)), "rQ": mix(u, ab[3]), "iQ": mix(v, cd[3]),
        "p1": ab[4] * d[2], "pr": cd[4] * (d[3] * (1 / RHO)),
        "n22a": ab[5] * per_block(1.0, RHO), "n22b": cd[5] * per_block(RHO, 1.0),
        "n11a": ab[6], "n11b": cd[6],
    }


def _write_plan(nb, spb):
    plan, step, sent = {}, WRITE_FROM, 0
    for b in range(nb):
        first = 0
        for n in WRITE_TAIL.get(b, (spb,)):
            ready = b * spb + first + n - 1
            if n == 1:
                copies = [(b, None, first, 1)]
            else:
                copies = [(b, p, c, 2) for p in range(8) for c in range(first, first + n, 2)]
            for copy in copies:
                step = max(step, ready, WRITE_FROM + sent // 8 - 1)
                sent += 4 if n == 1 else 1
                plan.setdefault(min(step, nb * spb - 1), []).append(copy)
            first += n
        assert first == spb
    return plan


def _kernel(x_hbm, w_hbm, b_hbm, o_hbm,
            xbuf, obuf, wbuf, bbuf, wt, lhs, lhs_diag, bias, xscale, xsem, wsem, osem):
    NB, NK, _, _, S = x_hbm.shape
    D, F = w_hbm.shape
    H = F // 2
    SPB = S // CH
    ALL = slice(None)

    def steps(first, n):
        return pl.ds(first * CH, n * CH)

    def xstart(sem, *idx, priority=0):
        pltpu.make_async_copy(x_hbm.at[idx], xbuf.at[idx], xsem.at[sem]).start(priority=priority)

    def xwait(sem, *idx):
        pltpu.make_async_copy(xbuf.at[idx], xbuf.at[idx], xsem.at[sem]).wait()

    def ring(bi):
        return jnp.where(bi >= RING, bi - RING, bi)

    def ostart(bi, phase, first, n):
        idx = (ALL, ALL if phase is None else phase, ALL, steps(first, n))
        pltpu.make_async_copy(
            obuf.at[(ring(bi),) + idx], o_hbm.at[(bi,) + idx], osem.at[ring(bi)]).start()

    def owait(slot):
        pltpu.make_async_copy(obuf.at[slot], obuf.at[slot], osem.at[slot]).wait()

    def wcopy(i, first, n):
        rows = pl.ds(first, n)
        return pltpu.make_async_copy(w_hbm.at[rows], wbuf.at[rows], wsem.at[i])

    bcopy = pltpu.make_async_copy(b_hbm, bbuf, wsem.at[5])
    bcopy.start()
    wcopy(4, 512, KB).start()

    @pl.loop(0, 4)
    def _(i):
        j = (i & 1) * 2 + (i >> 1)
        wcopy(j, pl.multiple_of(128 * j, 128), 128).start()

    xstart(3, 0, ALL, ALL, ALL, steps(0, GROUP))
    for p in range(4):
        xstart(0, 0, ALL, p, ALL, steps(GROUP, GROUP), priority=1)
    for p in range(4):
        xstart(1, 0, ALL, p, ALL, steps(UNIT, UNIT), priority=1)
    bg = PACED // SPB

    @pl.loop(0, 8)
    def _(p):
        for cond, b0 in ((p >= PACED_EXTRA, bg), (p < PACED_EXTRA, bg + 1)):
            pl.when(cond)(
                lambda: xstart(2, pl.ds(b0, NB - b0), ALL, p, ALL, steps(0, UNIT), priority=1))
        xstart(2, pl.ds(bg, NB - bg), ALL, p, ALL, steps(UNIT, UNIT), priority=1)

    bcopy.wait()
    bias[...] = jnp.broadcast_to(bbuf[...].reshape(1, F).astype(jnp.float32), (128, F)).T
    d, inv_d = {}, {}
    for i in (4, 0, 2, 1, 3):
        n = min(128, D - 128 * i)
        wcopy(i, 128 * i, n).wait()
        wp = _prune(wbuf[pl.ds(128 * i, n), :])
        tile = jnp.concatenate([wp] * (128 // n), axis=0).T
        wt[i] = _to_words(tile)
        if i < 4:
            d[i], inv_d[i] = _row_scale(tile)
            xscale[pl.ds(128 * i, 128)] = jnp.broadcast_to(d[i], (128, 128)).T
    for r in range(0, H // 2, 16):
        left = []
        for first in (r, H // 2 + r):
            upper, lower = (
                [_from_words(wt[i, pl.ds((h + first) // 2, 8)]).astype(jnp.float32) for i in range(5)]
                for h in (0, H))
            left.append(_left_operands(upper, lower, d, inv_d))
            for i, p in enumerate(PASSES):
                lhs[i, pl.ds(first // 2, 8)] = _to_words(left[-1][p])
        for k, n in enumerate(DIAG):
            terms = _strassen_left(*[part[n + ab] for part in left for ab in "ab"])
            for i, term in enumerate(terms):
                lhs_diag[7 * k + i, pl.ds(r // 2, 8)] = _to_words(term)

    def dot(left, right):
        return jnp.dot(_from_words(left), right.astype(jnp.bfloat16),
                       preferred_element_type=jnp.float32)

    def right_operand(bi, step, product):
        def halves(k):
            v = xbuf[bi, k, :, :, steps(step, 1)].astype(jnp.float32).reshape(KB, CH)
            return v[:, :128], v[:, 128:]

        n, i = product
        if n == 8:
            return halves(8)[i]
        (x11, x12), (x21, x22) = halves(n), halves(4 + n)
        d1, d2 = xscale[pl.ds(KB * n, KB)], xscale[pl.ds(KB * (4 + n), KB)]
        over_t = (lambda v: v) if T_SCALE[n] == 1.0 else (lambda v: v * (1 / T_SCALE[n]))
        return (x11 * d1 - over_t(x22 * d2), x11, x12 * d1 - x22 * d2, x21 * d2 - x11 * d1, x22,
                (x11 - over_t(x12)) * d1, (x21 - over_t(x22)) * d2)[i]

    plan = _write_plan(NB, SPB)
    span = UNROLL * SPB

    def start_writes(t, step):
        runs = [[(b - 2 * UNROLL * it, *rest) for b, *rest in plan.get(it * span + step, ())]
                for it in range(NB // UNROLL)]
        lo = 0
        for hi, run in enumerate(runs):
            if hi + 1 < len(runs) and runs[hi + 1] == run:
                continue
            if run:
                @pl.when((t >= lo) & (t <= hi))
                def _():
                    for db, *rest in run:
                        ostart(2 * UNROLL * t + db, *rest)
            lo = hi + 1

    def group(t, u, g):
        bi = t * UNROLL + u
        here = bi * SPB + g
        top = u == 0 and g == 0
        if top:
            pl.when(t == 0)(lambda: xwait(3, 0, ALL, ALL, ALL, steps(0, GROUP)))
        if u == 0 and g == GROUP:
            pl.when(t == 0)(lambda: xwait(0, 0, ALL, ALL, ALL, steps(GROUP, GROUP)))
        if g % UNIT == 0:
            pl.when((here > 0) & (here < PACED))(
                lambda: xwait(g // UNIT, bi, ALL, ALL, ALL, steps(g, UNIT)))
            if u * SPB + g == PACED % span:
                pl.when(here == PACED)(lambda: xwait(2, pl.ds(bg, NB - bg)))
            ahead = [(g + UNIT, p) for p in range(2, 6)]
        else:
            ahead = [(g + GROUP, 6), (g + GROUP, 7), (g + GROUP + UNIT, 0), (g + GROUP + UNIT, 1)]
        if g == 0:
            pl.when(bi >= RING)(lambda: owait(bi - RING))
        todo = [(c, p, k) for c, p in ahead for k in range(NK)]
        rows_done, total = [0], len(todo)

        def fetch(rows):
            rows_done[0] += rows
            while (total - len(todo)) * (3 * GROUP * H + 7 * H // 2) < rows_done[0] * total:
                i = total - len(todo)
                c, p, k = todo.pop(0)
                step = bi * SPB + c
                wanted = step < PACED + (p < PACED_EXTRA)
                if top and p < 4:
                    wanted = wanted & (t > 0)
                    if i % 3 != 2:
                        q = i - i // 3
                        pl.when(t == 0)(lambda: xstart(
                            0, 0, pl.ds(q % 3 * 3, 3), 4 + q // 3, ALL, steps(GROUP, GROUP)))
                pl.when(wanted)(lambda: xstart(
                    jnp.where(step < PACED, c // UNIT % 2, 2),
                    bi + c // SPB, k, p, ALL, steps(c % SPB, UNIT)))

        def right_tiles(rows, build):
            half = {}
            for h in (1, 0):
                fetch(rows // 2)
                half[h] = build(h)
            return [jnp.concatenate(pair, axis=0) for pair in zip(half[0], half[1])]

        def passes(e, *names):
            right = right_tiles(
                H, lambda h: [right_operand(bi, g + e, PRODUCTS[p][h]) for p in names])
            return [dot(lhs[PASSES.index(p)], r) for p, r in zip(names, right)]

        last_passes = {0: passes(0, "p1", "pr", "q1", "qr")} if top else {}
        diag = {}
        for e in range(0, GROUP, 2):
            for k, n in enumerate(DIAG):
                right = right_tiles(7 * H // 8, lambda h: _strassen_right(*[
                    right_operand(bi, g + e + d, PRODUCTS[n + ab][h]) for ab in "ab" for d in (0, 1)]))
                m = {i: dot(lhs_diag[7 * k + i], right[i]) for i in (0, 3, 4, 6, 2, 1, 5)}
                diag[n, e] = jnp.concatenate([(m[0] + m[3]) + (m[4] + m[6]), m[1] + m[3]], axis=0)
                diag[n, e + 1] = jnp.concatenate([m[2] + m[4], (m[1] - m[0]) + (m[2] - m[5])], axis=0)

        for e in range(GROUP):
            m1q, mrq, miq, phi = passes(e, "1Q", "rQ", "iQ", "phi")
            c11 = (m1q + mrq) + (miq + phi) + diag["n11", e]
            c21 = m1q + mrq * RHO + miq * (1 / RHO)
            minus_c22 = diag["n22", e] + phi
            m1p, mrp, mip, psi = passes(e, "1P", "rP", "iP", "psi")
            c12 = m1p + mrp + mip
            c22 = (m1p - minus_c22) + (mrp - psi) * RHO + mip * (1 / RHO)
            mp1, mpr, mq1, mqr = last_passes.get(e) or passes(e, "p1", "pr", "q1", "qr")
            b1, b2 = bias[0:H], bias[H:F]
            c12 = (c12 + b1) + mp1 + mpr * RHO
            c11 = ((c11 + psi) + b1) + (mp1 + mpr)
            c21 = (c21 + b2) + (mq1 + mqr)
            c22 = (c22 + b2) + (mq1 + mqr * RHO)
            for r0, quadrants in ((0, (c11, c12)), (H, (c21, c22))):
                val = jnp.concatenate(quadrants, axis=1)
                for k in range(r0 // KB, (r0 + H - 1) // KB + 1):
                    lo, hi = max(r0, KB * k), min(r0 + H, KB * (k + 1))
                    part = val[lo - r0:hi - r0].reshape((hi - lo) // 8, 8, CH)
                    phases = pl.ds(lo % KB // 8, (hi - lo) // 8)
                    obuf[ring(bi), k, phases, :, steps(g + e, 1)] = part.astype(obuf.dtype)
            start_writes(t, u * SPB + g + e)
        assert not todo

    @pl.loop(0, NB // UNROLL)
    def _(t):
        for u in range(UNROLL):
            for g in range(0, SPB, GROUP):
                group(t, u, g)

    for bi in range(NB - RING, NB):
        owait(bi % RING)


@jax.jit
def pallas_standalone__structured_sparse_n_m__ragged_kernel(
    x: jax.Array,
    w: jax.Array,
    b: jax.Array,
):
    B, S, D = x.shape
    F = w.shape[1]
    out = pl.pallas_call(
        _kernel,
        in_specs=[pl.BlockSpec(memory_space=pl.ANY)] * 3,
        out_specs=pl.BlockSpec(memory_space=pl.ANY),
        out_shape=jax.ShapeDtypeStruct((B, F // KB, 8, 8, S), x.dtype),
        scratch_shapes=[
            pltpu.VMEM((B, D // KB, 8, 8, S), x.dtype),
            pltpu.VMEM((RING, F // KB, 8, 8, S), x.dtype),
            pltpu.VMEM((D, F), w.dtype),
            pltpu.VMEM((F,), b.dtype),
            pltpu.VMEM((5, F // 2, 128), jnp.int32),
            pltpu.VMEM((len(PASSES), F // 4, 128), jnp.int32),
            pltpu.VMEM((7 * len(DIAG), F // 8, 128), jnp.int32),
            pltpu.VMEM((F, 128), jnp.float32),
            pltpu.VMEM((8 * KB, 128), jnp.float32),
            pltpu.SemaphoreType.DMA((4,)),
            pltpu.SemaphoreType.DMA((6,)),
            pltpu.SemaphoreType.DMA((RING,)),
        ],
        compiler_params=pltpu.CompilerParams(
            vmem_limit_bytes=126 * 1024 * 1024,
            disable_bounds_checks=True,
            disable_semaphore_checks=True,
            flags={"XLA_TPU_RESCHEDULE_DMA_DONES": True, "XLA_TPU_MAX_INSTS_TO_PREDICATE": 65536},
        ),
    )(jnp.transpose(x, (0, 2, 1)).reshape(B, D // KB, 8, 8, S), w, b)
    return jnp.transpose(out.reshape(B, F, S), (0, 2, 1))
```

```python
import jax
import jax.numpy as jnp
from jax import lax
import jax.experimental.pallas as pl
import jax.experimental.pallas.tpu as pltpu

KB = 64
CH = 256
GROUP = 4
UNIT = 8
UNROLL = 2

RHO = 2.0
T_SCALE = (1.0, 1.0, RHO, RHO)
PASSES = ("1Q", "rQ", "iQ", "phi", "1P", "rP", "iP", "psi", "p1", "pr", "q1", "qr")
DIAG = ("n11", "n22")
PRODUCTS = {
    "phi": ((0, 0), (3, 0)), "psi": ((2, 0), (1, 0)),
    "q1": ((0, 1), (1, 1)), "qr": ((2, 1), (3, 1)),
    "1P": ((0, 2), (2, 2)), "rP": ((8, 1), (1, 2)), "iP": ((8, 1), (3, 2)),
    "1Q": ((0, 3), (2, 3)), "rQ": ((8, 0), (1, 3)), "iQ": ((8, 0), (3, 3)),
    "p1": ((0, 4), (1, 4)), "pr": ((2, 4), (3, 4)),
    "n22a": ((0, 5), (1, 5)), "n22b": ((2, 5), (3, 5)),
    "n11a": ((0, 6), (1, 6)), "n11b": ((2, 6), (3, 6)),
}

MAX_CANCELLATION = 0.45

PACED = 128
PACED_EXTRA = 4
WRITE_FROM = 122
WRITE_TAIL = {14: (14, 2), 15: (6, 4, 2, 1, 1, 1, 1)}
RING = 9


def _prune_packed(u):
    mate = lax.broadcasted_iota(jnp.int32, u.shape, 0) ^ 1
    lo = pltpu.bitcast((u << 16) & 0x7FFFFFFF, jnp.float32)
    hi = pltpu.bitcast(u & 0x7FFF0000, jnp.float32)
    big, small = jnp.maximum(lo, hi), jnp.minimum(lo, hi)
    nbig = jnp.take_along_axis(big, mate, axis=0, mode="promise_in_bounds")
    nsmall = jnp.take_along_axis(small, mate, axis=0, mode="promise_in_bounds")
    thr = jnp.maximum(jnp.minimum(big, nbig), jnp.maximum(small, nsmall))
    return u & (jnp.where(lo < thr, 0, 0xFFFF) | jnp.where(hi < thr, 0, -65536))


def _prune(w):
    u = pltpu.bitcast(w, jnp.int32)
    parts = [_prune_packed(u[8 * i:8 * i + 8]) for i in range(u.shape[0] // 8)]
    return pltpu.bitcast(jnp.concatenate(parts, axis=0), jnp.bfloat16)


def _strassen_left(a11, a12, a21, a22):
    return [a11 + a22, a21 + a22, a11, a22, a11 + a12, a21 - a11, a12 - a22]


def _strassen_right(b11, b12, b21, b22):
    return [b11 - b22, b11, b12 - b22, b21 - b11, b22, b11 - b12, b21 - b22]


def _to_words(v):
    return pltpu.bitcast(v.astype(jnp.bfloat16), jnp.int32)


def _from_words(u):
    return pltpu.bitcast(u, jnp.bfloat16)


def _row_scale(wt):
    largest = jnp.max(jnp.abs(wt.astype(jnp.float32)), axis=0, keepdims=True)
    exponent = jnp.clip(pltpu.bitcast(largest, jnp.int32) >> 23, 2, 252)
    d = pltpu.bitcast(exponent << 23, jnp.float32)
    return jnp.where(largest == 0.0, 0.0, d), pltpu.bitcast((254 - exponent) << 23, jnp.float32)


def _left_operands(upper, lower, d, inv_d):
    low = lax.broadcasted_iota(jnp.int32, upper[0].shape, 1) < KB
    mix = lambda a, b: jnp.where(low, a, b)
    per_block = lambda a, b: jnp.where(low[0:1], a, b)
    ab, cd = [
        _strassen_left(upper[i] * inv_d[i], upper[i + 2] * inv_d[i + 2],
                       lower[i] * (inv_d[i] * inv_s), lower[i + 2] * (inv_d[i + 2] * inv_s))
        for i, inv_s in enumerate((per_block(1.0, 1 / RHO), per_block(1.0, RHO)))]
    u = (lower[4] - upper[4] * (1 / RHO)) * (1 / (RHO - 1 / RHO))
    v = (upper[4] * RHO - lower[4]) * (1 / (RHO - 1 / RHO))
    return {
        "phi": mix(ab[0], cd[0]), "psi": mix(cd[0], ab[0]),
        "q1": ab[1] * (d[0] * per_block(1.0, RHO)), "qr": cd[1] * (d[1] * per_block(1.0, 1 / RHO)),
        "1P": mix(ab[2], pltpu.roll(cd[2], KB, 1)), "rP": mix(u, ab[2]), "iP": mix(v, cd[2]),
        "1Q": mix(ab[3], pltpu.roll(cd[3], KB, 1)), "rQ": mix(u, ab[3]), "iQ": mix(v, cd[3]),
        "p1": ab[4] * d[2], "pr": cd[4] * (d[3] * (1 / RHO)),
        "n22a": ab[5] * per_block(1.0, RHO), "n22b": cd[5] * per_block(RHO, 1.0),
        "n11a": ab[6], "n11b": cd[6],
    }


def _write_plan(nb, spb):
    plan, step, sent = {}, WRITE_FROM, 0
    for b in range(nb):
        first = 0
        for n in WRITE_TAIL.get(b, (spb,)):
            ready = b * spb + first + n - 1
            if n == 1:
                copies = [(b, None, first, 1)]
            else:
                copies = [(b, p, c, 2) for p in range(8) for c in range(first, first + n, 2)]
            for copy in copies:
                step = max(step, ready, WRITE_FROM + sent // 8 - 1)
                sent += 4 if n == 1 else 1
                plan.setdefault(min(step, nb * spb - 1), []).append(copy)
            first += n
        assert first == spb
    return plan


def _kernel(x_hbm, w_hbm, b_hbm, o_hbm,
            xbuf, obuf, wbuf, bbuf, wt, lhs, lhs_diag, bias, xscale, xsem, wsem, osem):
    NB, NK, _, _, S = x_hbm.shape
    D, F = w_hbm.shape
    H = F // 2
    SPB = S // CH
    ALL = slice(None)

    def steps(first, n):
        return pl.ds(first * CH, n * CH)

    def xstart(sem, *idx, priority=0):
        pltpu.make_async_copy(x_hbm.at[idx], xbuf.at[idx], xsem.at[sem]).start(priority=priority)

    def xwait(sem, *idx):
        pltpu.make_async_copy(xbuf.at[idx], xbuf.at[idx], xsem.at[sem]).wait()

    def ring(bi):
        return jnp.where(bi >= RING, bi - RING, bi)

    def ostart(bi, phase, first, n):
        idx = (ALL, ALL if phase is None else phase, ALL, steps(first, n))
        pltpu.make_async_copy(
            obuf.at[(ring(bi),) + idx], o_hbm.at[(bi,) + idx], osem.at[ring(bi)]).start()

    def owait(slot):
        pltpu.make_async_copy(obuf.at[slot], obuf.at[slot], osem.at[slot]).wait()

    def wcopy(i, first, n):
        rows = pl.ds(first, n)
        return pltpu.make_async_copy(w_hbm.at[rows], wbuf.at[rows], wsem.at[i])

    bcopy = pltpu.make_async_copy(b_hbm, bbuf, wsem.at[5])
    bcopy.start()
    wcopy(4, 512, KB).start()

    @pl.loop(0, 4)
    def _(i):
        j = (i & 1) * 2 + (i >> 1)
        wcopy(j, pl.multiple_of(128 * j, 128), 128).start()

    xstart(3, 0, ALL, ALL, ALL, steps(0, GROUP))
    for p in range(4):
        xstart(0, 0, ALL, p, ALL, steps(GROUP, GROUP), priority=1)
    for p in range(4):
        xstart(1, 0, ALL, p, ALL, steps(UNIT, UNIT), priority=1)
    bg = PACED // SPB

    @pl.loop(0, 8)
    def _(p):
        for cond, b0 in ((p >= PACED_EXTRA, bg), (p < PACED_EXTRA, bg + 1)):
            pl.when(cond)(
                lambda: xstart(2, pl.ds(b0, NB - b0), ALL, p, ALL, steps(0, UNIT), priority=1))
        xstart(2, pl.ds(bg, NB - bg), ALL, p, ALL, steps(UNIT, UNIT), priority=1)

    bcopy.wait()
    bias[...] = jnp.broadcast_to(bbuf[...].reshape(1, F).astype(jnp.float32), (128, F)).T
    d, inv_d = {}, {}
    for i in (4, 0, 2, 1, 3):
        n = min(128, D - 128 * i)
        wcopy(i, 128 * i, n).wait()
        wp = _prune(wbuf[pl.ds(128 * i, n), :])
        tile = jnp.concatenate([wp] * (128 // n), axis=0).T
        wt[i] = _to_words(tile)
        d[i], inv_d[i] = _row_scale(tile)
        xscale[pl.ds(128 * i, n)] = jnp.broadcast_to(d[i], (128, 128)).T[:n]
    for r in range(0, H // 2, 16):
        left = []
        for first in (r, H // 2 + r):
            upper, lower = (
                [_from_words(wt[i, pl.ds((h + first) // 2, 8)]).astype(jnp.float32) for i in range(5)]
                for h in (0, H))
            left.append(_left_operands(upper, lower, d, inv_d))
            for i, p in enumerate(PASSES):
                lhs[i, pl.ds(first // 2, 8)] = _to_words(left[-1][p])
        for k, n in enumerate(DIAG):
            terms = _strassen_left(*[part[n + ab] for part in left for ab in "ab"])
            for i, term in enumerate(terms):
                lhs_diag[7 * k + i, pl.ds(r // 2, 8)] = _to_words(term)

    def dot(left, right):
        return jnp.dot(_from_words(left), right.astype(jnp.bfloat16),
                       preferred_element_type=jnp.float32)

    def right_operand(bi, step, product, scaled):
        def halves(k):
            v = xbuf[bi, k, :, :, steps(step, 1)].astype(jnp.float32).reshape(KB, CH)
            return v[:, :128], v[:, 128:]

        n, i = product
        if n == 8:
            scaled[8] = halves(8)[i] * xscale[pl.ds(KB * 8, KB)]
            return halves(8)[i]
        (x11, x12), (x21, x22) = halves(n), halves(4 + n)
        d1, d2 = xscale[pl.ds(KB * n, KB)], xscale[pl.ds(KB * (4 + n), KB)]
        if i in (2, 3):
            scaled[n], scaled[4 + n] = (x12 * d1, x22 * d2) if i == 2 else (x11 * d1, x21 * d2)
        over_t = (lambda v: v) if T_SCALE[n] == 1.0 else (lambda v: v * (1 / T_SCALE[n]))
        return (x11 * d1 - over_t(x22 * d2), x11, x12 * d1 - x22 * d2, x21 * d2 - x11 * d1, x22,
                (x11 - over_t(x12)) * d1, (x21 - over_t(x22)) * d2)[i]

    plan = _write_plan(NB, SPB)
    span = UNROLL * SPB

    def start_writes(t, step):
        runs = [[(b - 2 * UNROLL * it, *rest) for b, *rest in plan.get(it * span + step, ())]
                for it in range(NB // UNROLL)]
        lo = 0
        for hi, run in enumerate(runs):
            if hi + 1 < len(runs) and runs[hi + 1] == run:
                continue
            if run:
                @pl.when((t >= lo) & (t <= hi))
                def _():
                    for db, *rest in run:
                        ostart(2 * UNROLL * t + db, *rest)
            lo = hi + 1

    def group(t, u, g, level):
        bi = t * UNROLL + u
        here = bi * SPB + g
        top = u == 0 and g == 0
        if top:
            pl.when(t == 0)(lambda: xwait(3, 0, ALL, ALL, ALL, steps(0, GROUP)))
        if u == 0 and g == GROUP:
            pl.when(t == 0)(lambda: xwait(0, 0, ALL, ALL, ALL, steps(GROUP, GROUP)))
        if g % UNIT == 0:
            pl.when((here > 0) & (here < PACED))(
                lambda: xwait(g // UNIT, bi, ALL, ALL, ALL, steps(g, UNIT)))
            if u * SPB + g == PACED % span:
                pl.when(here == PACED)(lambda: xwait(2, pl.ds(bg, NB - bg)))
            ahead = [(g + UNIT, p) for p in range(2, 6)]
        else:
            ahead = [(g + GROUP, 6), (g + GROUP, 7), (g + GROUP + UNIT, 0), (g + GROUP + UNIT, 1)]
        if g == 0:
            pl.when(bi >= RING)(lambda: owait(bi - RING))
        todo = [(c, p, k) for c, p in ahead for k in range(NK)]
        rows_done, total = [0], len(todo)

        def fetch(rows):
            rows_done[0] += rows
            while (total - len(todo)) * (3 * GROUP * H + 7 * H // 2) < rows_done[0] * total:
                i = total - len(todo)
                c, p, k = todo.pop(0)
                step = bi * SPB + c
                wanted = step < PACED + (p < PACED_EXTRA)
                if top and p < 4:
                    wanted = wanted & (t > 0)
                    if i % 3 != 2:
                        q = i - i // 3
                        pl.when(t == 0)(lambda: xstart(
                            0, 0, pl.ds(q % 3 * 3, 3), 4 + q // 3, ALL, steps(GROUP, GROUP)))
                pl.when(wanted)(lambda: xstart(
                    jnp.where(step < PACED, c // UNIT % 2, 2),
                    bi + c // SPB, k, p, ALL, steps(c % SPB, UNIT)))

        def right_tiles(rows, build):
            half = {}
            for h in (1, 0):
                fetch(rows // 2)
                half[h] = build(h)
            return [jnp.concatenate(pair, axis=0) for pair in zip(half[0], half[1])]

        def passes(e, *names):
            scaled = {}
            right = right_tiles(
                H, lambda h: [right_operand(bi, g + e, PRODUCTS[p][h], scaled) for p in names])
            if scaled:
                blocks, rows = list(scaled.values()), []
                for part in (blocks[:6], blocks[6:]):
                    for r in reversed(range(0, KB, 8)):
                        squares = [v[r:r + 8] * v[r:r + 8] for v in part]
                        rows.append(sum(squares[1:], squares[0]))
                energy = jnp.sum(sum(rows[1:], rows[0]), axis=0, keepdims=True)
                level["energy"] = jnp.maximum(level["energy"], energy)
            return [dot(lhs[PASSES.index(p)], r) for p, r in zip(names, right)]

        last_passes = {0: passes(0, "p1", "pr", "q1", "qr")} if top else {}
        diag = {}
        for e in range(0, GROUP, 2):
            for k, n in enumerate(DIAG):
                right = right_tiles(7 * H // 8, lambda h: _strassen_right(*[
                    right_operand(bi, g + e + j, PRODUCTS[n + ab][h], {})
                    for ab in "ab" for j in (0, 1)]))
                m = {i: dot(lhs_diag[7 * k + i], right[i]) for i in (0, 3, 4, 6, 2, 1, 5)}
                diag[n, e] = jnp.concatenate([(m[0] + m[3]) + (m[4] + m[6]), m[1] + m[3]], axis=0)
                diag[n, e + 1] = jnp.concatenate([m[2] + m[4], (m[1] - m[0]) + (m[2] - m[5])], axis=0)

        for e in range(GROUP):
            m1q, mrq, miq, phi = passes(e, "1Q", "rQ", "iQ", "phi")
            c11 = (m1q + mrq) + (miq + phi) + diag["n11", e]
            c21 = m1q + mrq * RHO + miq * (1 / RHO)
            minus_c22 = diag["n22", e] + phi
            m1p, mrp, mip, psi = passes(e, "1P", "rP", "iP", "psi")
            c12 = m1p + mrp + mip
            c22 = (m1p - minus_c22) + (mrp - psi) * RHO + mip * (1 / RHO)
            mp1, mpr, mq1, mqr = last_passes.get(e) or passes(e, "p1", "pr", "q1", "qr")
            b1, b2 = bias[0:H], bias[H:F]
            c12 = (c12 + b1) + mp1 + mpr * RHO
            c11 = ((c11 + psi) + b1) + (mp1 + mpr)
            c21 = (c21 + b2) + (mq1 + mqr)
            c22 = (c22 + b2) + (mq1 + mqr * RHO)
            sample = 16 * (u * SPB + g + e) % H
            for c in (c11, c12, c21, c22):
                level["peak"] = jnp.maximum(level["peak"], jnp.abs(c[sample:sample + 16]))
            for r0, quadrants in ((0, (c11, c12)), (H, (c21, c22))):
                val = jnp.concatenate(quadrants, axis=1)
                for k in range(r0 // KB, (r0 + H - 1) // KB + 1):
                    lo, hi = max(r0, KB * k), min(r0 + H, KB * (k + 1))
                    part = val[lo - r0:hi - r0].reshape((hi - lo) // 8, 8, CH)
                    phases = pl.ds(lo % KB // 8, (hi - lo) // 8)
                    obuf[ring(bi), k, phases, :, steps(g + e, 1)] = part.astype(obuf.dtype)
            start_writes(t, u * SPB + g + e)
        assert not todo

    def body(t, level):
        level = dict(level)
        for u in range(UNROLL):
            for g in range(0, SPB, GROUP):
                group(t, u, g, level)
        return level

    level = lax.fori_loop(0, NB // UNROLL, body, {
        "energy": jnp.zeros((1, 128), jnp.float32), "peak": jnp.zeros((16, 128), jnp.float32)})

    unit = [_from_words(wt[i]).astype(jnp.float32) * inv_d[i] for i in range(5)]
    squares = sum((v * v for v in unit[:4]), unit[4] * unit[4] * 0.5)
    weight = jnp.max(jnp.sum(squares, axis=1, keepdims=True), axis=0, keepdims=True) * (1 / D)
    peak = jnp.max(jnp.max(level["peak"], axis=1, keepdims=True), axis=0, keepdims=True)
    fine = level["energy"] * weight <= jnp.square(peak * MAX_CANCELLATION)
    fine = fine & (peak >= 1e-15) & (peak <= 1e15)
    redo = jnp.max(jnp.where(fine, 0, 1)) > 0

    pl.loop(NB - RING, NB)(lambda bi: owait(ring(bi)))

    @pl.when(redo)
    def _():
        @pl.loop(0, NB)
        def _(bi):
            @pl.loop(0, SPB)
            def _(step):
                cols = pl.ds(pl.multiple_of(step * CH, CH), CH)
                x = xbuf[bi, :, :, :, cols].astype(jnp.float32).reshape(D, CH)
                acc = jnp.dot(_from_words(wt[4])[:, :KB], x[8 * KB:].astype(jnp.bfloat16),
                              preferred_element_type=jnp.float32)
                for i in range(4):
                    acc = acc + dot(wt[i], x[128 * i:128 * (i + 1)])
                acc = acc + jnp.concatenate([bias[...]] * (CH // 128), axis=1)
                obuf[0, :, :, :, cols] = acc.reshape(F // KB, 8, 8, CH).astype(obuf.dtype)

            copy = pltpu.make_async_copy(obuf.at[0], o_hbm.at[bi], osem.at[0])
            copy.start()
            copy.wait()


@jax.jit
def pallas_standalone__structured_sparse_n_m__ragged_kernel(
    x: jax.Array,
    w: jax.Array,
    b: jax.Array,
):
    B, S, D = x.shape
    F = w.shape[1]
    out = pl.pallas_call(
        _kernel,
        in_specs=[pl.BlockSpec(memory_space=pl.ANY)] * 3,
        out_specs=pl.BlockSpec(memory_space=pl.ANY),
        out_shape=jax.ShapeDtypeStruct((B, F // KB, 8, 8, S), x.dtype),
        scratch_shapes=[
            pltpu.VMEM((B, D // KB, 8, 8, S), x.dtype),
            pltpu.VMEM((RING, F // KB, 8, 8, S), x.dtype),
            pltpu.VMEM((D, F), w.dtype),
            pltpu.VMEM((F,), b.dtype),
            pltpu.VMEM((5, F // 2, 128), jnp.int32),
            pltpu.VMEM((len(PASSES), F // 4, 128), jnp.int32),
            pltpu.VMEM((7 * len(DIAG), F // 8, 128), jnp.int32),
            pltpu.VMEM((F, 128), jnp.float32),
            pltpu.VMEM((D, 128), jnp.float32),
            pltpu.SemaphoreType.DMA((4,)),
            pltpu.SemaphoreType.DMA((6,)),
            pltpu.SemaphoreType.DMA((RING,)),
        ],
        compiler_params=pltpu.CompilerParams(
            vmem_limit_bytes=126 * 1024 * 1024,
            disable_bounds_checks=True,
            disable_semaphore_checks=True,
            flags={"XLA_TPU_RESCHEDULE_DMA_DONES": True, "XLA_TPU_MAX_INSTS_TO_PREDICATE": 65536},
        ),
    )(jnp.transpose(x, (0, 2, 1)).reshape(B, D // KB, 8, 8, S), w, b)
    return jnp.transpose(out.reshape(B, F, S), (0, 2, 1))
```
